```python
import jax
import jax.numpy as jnp

def _softmax(x, axis=-1):
    return jax.nn.softmax(x, axis=axis)
def _gelu(x):
    return jax.nn.gelu(x, approximate=True)
def _silu(x):
    return jax.nn.silu(x)
def _sigmoid(x):
    return jax.nn.sigmoid(x)
def _layernorm(x, axis=-1, eps=1e-5):
    m = jnp.mean(x, axis=axis, keepdims=True)
    v = jnp.var(x, axis=axis, keepdims=True)
    return (x - m) / jnp.sqrt(v + eps)
def _scatter_add(tgt, idx, src, axis=0):
    return tgt.at[idx].add(src)
def _segment_sum(src, seg, n):
    return jax.ops.segment_sum(src, seg, n)
class _Rng:
    def __init__(self, key):
        self._k = key
    def _next(self):
        self._k, sub = jax.random.split(self._k)
        return sub
    def normal(self, shape):
        return jax.random.normal(self._next(), shape, dtype=jnp.bfloat16)
    def randint(self, lo, hi, shape):
        return jax.random.randint(self._next(), shape, lo, hi, dtype=jnp.int32)
    def uniform(self, shape, lo=0.0, hi=1.0):
        return jax.random.uniform(self._next(), shape, jnp.bfloat16, lo, hi)
    def permutation(self, n):
        return jax.random.permutation(self._next(), n)


kernel_name = 'interleave_layers__sliding_local_dilated__glu_gated_glu__prompt'

def setup_inputs():
    _rng = _Rng(jax.random.key(int.from_bytes(__import__("os").urandom(4), "little")))
    _w = (lambda a: (lambda t: t.astype(jnp.bfloat16) if jnp.issubdtype(t.dtype, jnp.floating) else t)(jnp.asarray(a)))
    def _A_setup():
        B, S, D = 1, 2048, 576
        return {
            "x": _w((lambda *s: _rng.normal(s) * 0.05)(B, S, D)),
            "wqkv": _w((lambda *s: _rng.normal(s) * 0.05)(D, 3 * D)),
            "wo": _w((lambda *s: _rng.normal(s) * 0.05)(D, D)),
        }
    _A_in = _A_setup()

    def _B_setup():
        B, S, D, F = 1, 2048, 576, 4608
        return {
            "x": _w((lambda *s: _rng.normal(s) * 0.05)(B, S, D)),
            "w_gate": _w((lambda *s: _rng.normal(s) * 0.05)(D, F)),
            "w_up": _w((lambda *s: _rng.normal(s) * 0.05)(D, F)),
            "w_down": _w((lambda *s: _rng.normal(s) * 0.05)(F, D)),
        }
    _B_in = _B_setup()

    return {
        "A_x": _A_in["x"],
        "A_wqkv": _A_in["wqkv"],
        "A_wo": _A_in["wo"],
        "B_x": _B_in["x"],
        "B_w_gate": _B_in["w_gate"],
        "B_w_up": _B_in["w_up"],
        "B_w_down": _B_in["w_down"],
    }

def reference(A_x, A_wqkv, A_wo, B_x, B_w_gate, B_w_up, B_w_down):
    def _A_ref(x, wqkv, wo):
        B, S, D = x.shape
        H = 32; Dh = D // H
        W, dil = 8, 2
        qkv = (lambda x, *d: x.transpose(*d))((x @ wqkv).reshape(B, S, 3, H, Dh), 2, 0, 3, 1, 4)
        q, k, v = qkv[0], qkv[1], qkv[2]
        scale = Dh ** -0.5
        pos = jnp.arange(S)
        off = jnp.arange(W) * dil
        idx = pos[:, None] - off[None, :]
        mask = idx >= 0
        idx_c = jnp.where(mask, idx, 0).reshape(-1)
        kg = k[:, :, idx_c, :].reshape(B, H, S, W, Dh)
        vg = v[:, :, idx_c, :].reshape(B, H, S, W, Dh)
        logits = jnp.einsum("bhsd,bhswd->bhsw", q, kg) * scale
        logits = jnp.where(mask[None, None, :, :], logits, -1e9)
        attn = _softmax(logits, axis=-1)
        o = jnp.einsum("bhsw,bhswd->bhsd", attn, vg)
        return (lambda x, *d: x.transpose(*d))(o, 0, 2, 1, 3).reshape(B, S, D) @ wo

    def _B_ref(x, w_gate, w_up, w_down):
        g = jnp.einsum("bsd,df->bsf", x, w_gate)
        u = jnp.einsum("bsd,df->bsf", x, w_up)
        h = _sigmoid(g) * u
        return jnp.einsum("bsf,fd->bsd", h, w_down)

    x = A_x
    x = x + _A_ref(_layernorm(x, axis=-1), A_wqkv, A_wo)
    x = x + _B_ref(_layernorm(x, axis=-1), B_w_gate, B_w_up, B_w_down)
    x = x + _A_ref(_layernorm(x, axis=-1), A_wqkv, A_wo)
    x = x + _B_ref(_layernorm(x, axis=-1), B_w_gate, B_w_up, B_w_down)
    return x
```

```python
import jax
import jax.numpy as jnp
from jax import lax
import jax.experimental.pallas as pl
import jax.experimental.pallas.tpu as pltpu

S, D, F = 2048, 576, 4608
H, DH, W = 32, 18, 8
NB = 8
KT = (0, 128, 256, 384, 448)
NC = 3
FC = F // NC
FN = FC // 4
DQ = D // 4
DH2 = D // 2

f32 = jnp.float32
bf16 = jnp.bfloat16
u32 = jnp.uint32


def _dot(a, b):
    return jnp.dot(a, b, preferred_element_type=f32)


def _unpack_lo(w):
    return pltpu.bitcast(w << 16, f32)


def _unpack_hi(w):
    return pltpu.bitcast(w & u32(0xFFFF0000), f32)


def _a_sums(a11, a12, a21, a22):
    return (a11 + a22, a21 + a22, a11, a22, a11 + a12, a21 - a11, a12 - a22)


def _b_sums(b11, b12, b21, b22):
    return (b11 + b22, b11, b12 - b22, b21 - b11, b22, b11 + b12, b21 + b22)


def _c_sums(m):
    m1, m2, m3, m4, m5, m6, m7 = m
    return ((m1 + m4 - m5 + m7, m3 + m5), (m2 + m4, m1 - m2 + m3 + m6))


def _prep_weights(quarters, a_ref, az_ref, rows):
    lo = lax.broadcasted_iota(jnp.int32, quarters[0][0].shape, 1) < 64
    w = [[None, None], [None, None]]
    for x in range(2):
        t1, t2 = quarters[2 * x], quarters[2 * x + 1]
        w[0][x] = t1[:3] + [jnp.where(lo, t1[3], t1[3] - t2[3])]
        w[1][x] = t2[:3] + [jnp.where(lo, t2[3], t2[4] - t1[4])]
        az_ref[x, rows, :] = jnp.where(lo, t2[4], t1[4]).astype(bf16)
    for ty in range(2):
        wa, wb = w[ty]
        for k in range(2):
            for p, s in enumerate(_a_sums(wa[k], wa[2 + k], wb[k], wb[2 + k])):
                a_ref[ty, p, rows, 128 * k:128 * (k + 1)] = s.astype(bf16)


def _prep_acts(xn, bs_ref, bz_ref):
    t1, t2 = xn[:, 0:128], xn[:, 128:256]
    for p, s in enumerate(_b_sums(t1[0:256], t2[0:256], t1[256:512], t2[256:512])):
        bs_ref[p, 0:256, :] = s.astype(bf16)
    for p, s in enumerate(_b_sums(t1[192:256], t2[192:256], t1[512:576], t2[512:576])):
        if p not in (1, 5):
            bs_ref[p, 256:320, :] = s.astype(bf16)
    bz_ref[...] = xn[448:576].astype(bf16)


def _matmul(a_ref, az_ref, rows, bs_ref, bz_ref):
    c = []
    for ty in range(2):
        m = []
        for p in range(7):
            if ty == 0 or p in (1, 5):
                b = bs_ref[p, 0:256, :]
            else:
                b = jnp.concatenate([bs_ref[p, 0:192, :], bs_ref[p, 256:320, :]], axis=0)
            m.append(_dot(a_ref[ty, p, rows, :], b))
        c.append(_c_sums(m))
    out = []
    for x in range(2):
        z = _dot(az_ref[x, rows, :], bz_ref[...])
        for ty in range(2):
            out.append([c[ty][x][t] + z[:, 128 * t:128 * (t + 1)] for t in range(2)])
    return out


def _layernorm(x):
    m = jnp.sum(x, axis=0, keepdims=True) * (1.0 / D)
    xc = x - m
    v = jnp.sum(xc * xc, axis=0, keepdims=True) * (1.0 / D)
    return xc * lax.rsqrt(v + 1e-5)


def _kernel(x_hbm, wqkv_hbm, wo_hbm, wg_hbm, wu_hbm, wd_hbm, out_hbm,
            xio, wqkv, wo, wg, wu, wd, sems,
            slab, wt,
            aq, azq, akv, azkv, ao, azo, agu, azgu, ad,
            x_ref, bs, bz, bso, bzo, k_ref, v_ref, q_ref):
    cp_qkv = pltpu.make_async_copy(wqkv_hbm, wqkv, sems.at[0])
    cp_x = pltpu.make_async_copy(x_hbm, xio, sems.at[1])
    cp_o = pltpu.make_async_copy(wo_hbm, wo, sems.at[2])
    cp_g = pltpu.make_async_copy(wg_hbm, wg, sems.at[3])
    cp_u = pltpu.make_async_copy(wu_hbm, wu, sems.at[4])
    cp_d = pltpu.make_async_copy(wd_hbm, wd, sems.at[5])
    cp_qkv.start()
    cp_x.start()
    cp_o.start()

    cp_qkv.wait()
    for k, r0 in enumerate(KT):
        slab[k, 0:3 * DH2, :] = pltpu.bitcast(wqkv[r0:r0 + 128, :].T, u32)
    for s in range(3):
        for k in range(5):
            for j in range(DH // 2):
                w2 = slab[k, pl.ds(s * DH2 + j, H, stride=DH // 2), :]
                wt[k, 64 * j:64 * j + 32, :] = _unpack_lo(w2)
                wt[k, 64 * j + 32:64 * j + 64, :] = _unpack_hi(w2)
        quarters = [[wt[k, DQ * i:DQ * (i + 1), :] for k in range(5)] for i in range(4)]
        if s == 0:
            _prep_weights(quarters, aq, azq, slice(0, DQ))
        else:
            _prep_weights(quarters, akv, azkv, slice(DQ * (s - 1), DQ * s))

    cp_x.wait()
    cp_g.start()
    cp_u.start()
    cp_d.start()
    for k, r0 in enumerate(KT):
        slab[k] = pltpu.bitcast(xio[r0:r0 + 128, :].T, u32)
    for c in range(NB):
        for k, r0 in enumerate(KT):
            w2 = slab[k, pl.ds(c, 128, stride=NB), :].T
            if k == 4:
                w2, r0 = w2[64:128], 512
            n = w2.shape[0]
            x_ref[c, r0:r0 + n, 0:128] = _unpack_lo(w2)
            x_ref[c, r0:r0 + n, 128:256] = _unpack_hi(w2)

    cp_o.wait()
    for n in range(5):
        wd_n = min(128, D - 128 * n)
        blk = pltpu.bitcast(wo[:, 128 * n:128 * n + wd_n], u32)
        if wd_n < 128:
            blk = jnp.concatenate([blk, blk], axis=1)
        slab[n, 0:DH2, :] = blk
        rows = []
        for j in range(DH // 2):
            w2 = slab[n, pl.ds(j, H, stride=DH // 2), :]
            rows += [_unpack_lo(w2), _unpack_hi(w2)]
        wp = jnp.concatenate(rows, axis=0)
        for k, r0 in enumerate(KT):
            wt[k, 128 * n:128 * n + wd_n, :] = wp[r0:r0 + 128].T[0:wd_n]
    _prep_weights([[wt[k, DQ * i:DQ * (i + 1), :] for k in range(5)] for i in range(4)],
                  ao, azo, slice(0, DQ))

    def layer(li, _):
        def kv_block(c, _):
            _prep_acts(_layernorm(x_ref[c]), bs.at[c], bz.at[c])
            out = _matmul(akv, azkv, slice(0, 2 * DQ), bs.at[c], bz.at[c])
            for i in range(4):
                for t in range(2):
                    for ref, o in ((k_ref, out[i][t][0:DQ]), (v_ref, out[i][t][DQ:2 * DQ])):
                        ref[t, c + NB, DQ * i:DQ * (i + 1), :] = o
                        ref[t, c, DQ * i:DQ * (i + 1), :] = pltpu.roll(o, 1, 1)
            return None

        lax.fori_loop(0, NB, kv_block, None)

        def attn_block(c, _):
            out = _matmul(aq, azq, slice(0, DQ), bs.at[c], bz.at[c])
            for i in range(4):
                for t in range(2):
                    q_ref[t, DQ * i:DQ * (i + 1), :] = out[i][t]
            lane = lax.broadcasted_iota(jnp.int32, (H, 128), 1)
            halves = []
            for t in range(2):
                logit = []
                for w in range(W):
                    acc = None
                    for d in range(DH):
                        rows = slice(H * d, H * (d + 1))
                        term = q_ref[t, rows, :] * k_ref[t, c + NB - w, rows, :]
                        acc = term if acc is None else acc + term
                    acc = acc * (DH ** -0.5)
                    if w > 0:
                        acc = jnp.where(lane * NB + (c - w) >= 0, acc, -1e9)
                    logit.append(acc)
                m = logit[0]
                for w in range(1, W):
                    m = jnp.maximum(m, logit[w])
                e = [jnp.exp(l - m) for l in logit]
                den = e[0]
                for w in range(1, W):
                    den = den + e[w]
                inv = 1.0 / den
                p = [x * inv for x in e]
                o = []
                for d in range(DH):
                    rows = slice(H * d, H * (d + 1))
                    acc = None
                    for w in range(W):
                        term = p[w] * v_ref[t, c + NB - w, rows, :]
                        acc = term if acc is None else acc + term
                    o.append(acc)
                halves.append(jnp.concatenate(o, axis=0))
            _prep_acts(jnp.concatenate(halves, axis=1), bso, bzo)
            out = _matmul(ao, azo, slice(0, DQ), bso, bzo)
            y = jnp.concatenate([jnp.concatenate(out[i], axis=1) for i in range(4)], axis=0)
            xnew = x_ref[c] + y
            x_ref[c] = xnew
            _prep_acts(_layernorm(xnew), bs.at[c], bz.at[c])
            return None

        lax.fori_loop(0, NB, attn_block, None)

        @pl.when(li == 0)
        def _():
            for cp, src, off in ((cp_g, wg, 0), (cp_u, wu, FN)):
                cp.wait()

                def prep(i, _):
                    j, r = i // (FN // 128), i % (FN // 128)
                    quarters = []
                    for qd in range(4):
                        c0 = pl.multiple_of(j * FC + qd * FN + r * 128, 128)
                        quarters.append([src[r0:r0 + 128, pl.ds(c0, 128)].T.astype(f32) * 0.5 for r0 in KT])
                    _prep_weights(quarters, agu, azgu,
                                  pl.ds(pl.multiple_of(j * 2 * FN + off + r * 128, 128), 128))
                    return None

                lax.fori_loop(0, NC * (FN // 128), prep, None)
            cp_d.wait()
            for j in range(NC):
                c1, c2 = slice(j * FC, j * FC + FC // 2), slice(j * FC + FC // 2, (j + 1) * FC)
                blocks = [wd[r, cc].astype(f32) for r in (slice(0, DH2), slice(DH2, D)) for cc in (c1, c2)]
                for p, s in enumerate(_a_sums(*blocks)):
                    ad[p, :, j * (FC // 2):(j + 1) * (FC // 2)] = s.astype(bf16)

        def ffn_block(c, _):
            acc = [None] * 7
            for j in range(NC):
                out = _matmul(agu, azgu, slice(2 * FN * j, 2 * FN * (j + 1)), bs.at[c], bz.at[c])
                h = [[o[FN:] + o[FN:] * jnp.tanh(o[:FN]) for o in oq] for oq in out]
                hb = [[jnp.concatenate([h[2 * x][t], h[2 * x + 1][t]], axis=0) for t in range(2)] for x in range(2)]
                for p, s in enumerate(_b_sums(hb[0][0], hb[0][1], hb[1][0], hb[1][1])):
                    m = _dot(ad[p, :, j * (FC // 2):(j + 1) * (FC // 2)], s.astype(bf16))
                    acc[p] = m if acc[p] is None else acc[p] + m
            y = _c_sums(acc)
            for x in range(2):
                for t in range(2):
                    x_ref[c, DH2 * x:DH2 * (x + 1), 128 * t:128 * (t + 1)] += y[x][t]
            return None

        lax.fori_loop(0, NB, ffn_block, None)
        return None

    lax.fori_loop(0, 2, layer, None)

    for c in range(NB):
        for k, r0 in enumerate(KT):
            ev = pltpu.bitcast(x_ref[c, r0:r0 + 128, 0:128].astype(bf16).astype(f32), u32)
            od = pltpu.bitcast(x_ref[c, r0:r0 + 128, 128:256].astype(bf16).astype(f32), u32)
            slab[k, pl.ds(c, 128, stride=NB), :] = ((ev >> 16) | od).T
    outs = []
    for k, r0 in enumerate(KT):
        blk = pltpu.bitcast(slab[k], bf16).T
        if k == 4:
            blk, r0 = blk[64:128], 512
        n = blk.shape[0]
        xio[r0:r0 + n, :] = blk
        cp = pltpu.make_async_copy(xio.at[r0:r0 + n], out_hbm.at[r0:r0 + n], sems.at[k])
        cp.start()
        outs.append(cp)
    for cp in outs:
        cp.wait()


@jax.jit
def pallas_interleave_layers__sliding_local_dilated__glu_gated_glu__prompt_kernel(
        A_x, A_wqkv, A_wo, B_x, B_w_gate, B_w_up, B_w_down):
    del B_x
    any_spec = pl.BlockSpec(memory_space=pl.ANY)
    V = pltpu.VMEM
    out = pl.pallas_call(
        _kernel,
        out_shape=jax.ShapeDtypeStruct((D, S), bf16),
        in_specs=[any_spec] * 6,
        out_specs=any_spec,
        scratch_shapes=[
            V((D, S), bf16), V((D, 3 * D), bf16), V((D, D), bf16),
            V((D, F), bf16), V((D, F), bf16), V((D, F), bf16),
            pltpu.SemaphoreType.DMA((6,)),
            V((5, S // 2, 128), u32), V((5, D, 128), f32),
            V((2, 7, DQ, 256), bf16), V((2, DQ, 128), bf16),
            V((2, 7, 2 * DQ, 256), bf16), V((2, 2 * DQ, 128), bf16),
            V((2, 7, DQ, 256), bf16), V((2, DQ, 128), bf16),
            V((2, 7, F // 2, 256), bf16), V((2, F // 2, 128), bf16),
            V((7, DH2, F // 2), bf16),
            V((NB, D, 256), f32),
            V((NB, 7, 320, 128), bf16), V((NB, 128, 256), bf16),
            V((7, 320, 128), bf16), V((128, 256), bf16),
            V((2, 2 * NB, D, 128), f32), V((2, 2 * NB, D, 128), f32), V((2, D, 128), f32),
        ],
        compiler_params=pltpu.CompilerParams(vmem_limit_bytes=120 * 2**20),
    )(A_x[0].T, A_wqkv, A_wo, B_w_gate, B_w_up, B_w_down.T)
    return out.T[None]
```

```python
import math

import jax
import jax.numpy as jnp
from jax import lax
import jax.experimental.pallas as pl
import jax.experimental.pallas.tpu as pltpu

S, D, F = 2048, 576, 4608
H, DH, W = 32, 18, 8
NCOL = 8
BC = 4
TB = 128 * BC
NBLK = S // TB
KT = (0, 128, 256, 384, 448)
UNIT = 512
NH = D // 64
AHEAD = 4
LA, LG, LD = 1, 2, 2
NG, A_STAT, A_ATT = 6, (1, 1, 0), (2, 1, 0)
ANC = 1
HIST = (5, 5, 5)
MODE = '-z'

f32 = jnp.float32
bf16 = jnp.bfloat16
u32 = jnp.uint32

X0 = 0
STAT0 = X0 + NBLK * BC * D
X_ROWS = STAT0 + 2 * BC * 2 * 8
QKV0 = 0
O0 = QKV0 + 2 * 5 * NCOL * D
P0 = O0 + BC * D
WORK_ROWS = P0 + BC * W * 8


def _dot(a, b):
    return jnp.dot(a, b, preferred_element_type=f32)


def _unpack_lo(w):
    return pltpu.bitcast(w << 16, f32)


def _unpack_hi(w):
    return pltpu.bitcast(w & u32(0xFFFF0000), f32)


def _load_bf16(ref, idx, row, n):
    return pltpu.bitcast(ref.bitcast(u32)[(*idx, slice(row // 2, (row + n) // 2))], bf16)


def _load_wide(ref, idx, row, n):
    return jnp.concatenate([_load_bf16(ref, (*idx, k), row, n) for k in range(ref.shape[len(idx)])], axis=1)


def _madd(a, b):
    return [[x + y for x, y in zip(r, s)] for r, s in zip(a, b)]


def _msub(a, b):
    return [[x - y for x, y in zip(r, s)] for r, s in zip(a, b)]


def _quad(m):
    n = len(m) // 2
    return ([r[:n] for r in m[:n]], [r[n:] for r in m[:n]], [r[:n] for r in m[n:]], [r[n:] for r in m[n:]])


def _a_sums(m):
    if len(m) == 1:
        yield m[0][0]
        return
    a11, a12, a21, a22 = _quad(m)
    yield from _a_sums(_madd(a11, a22))
    yield from _a_sums(_madd(a21, a22))
    yield from _a_sums(a11)
    yield from _a_sums(a22)
    yield from _a_sums(_madd(a11, a12))
    yield from _a_sums(_msub(a21, a11))
    yield from _a_sums(_msub(a12, a22))


def _b_sums(m):
    if len(m) == 1:
        yield m[0][0]
        return
    b11, b12, b21, b22 = _quad(m)
    yield from _b_sums(_madd(b11, b22))
    yield from _b_sums(b11)
    yield from _b_sums(_msub(b12, b22))
    yield from _b_sums(_msub(b21, b11))
    yield from _b_sums(b22)
    yield from _b_sums(_madd(b11, b12))
    yield from _b_sums(_madd(b21, b22))


def _c_sums(product, first, count, z=None):
    if count == 1:
        m = product(first)
        return [[m if z is None else m + z[0][0]]]
    k = count // 7
    zq = None if z is None else _quad(z)

    def az(i, m):
        return m if zq is None else _madd(m, zq[i])

    def g(i):
        return _c_sums(product, first + (i - 1) * k, k)

    m2 = g(2)
    m4 = g(4)
    c21 = _madd(az(2, m2), m4)
    m3 = g(3)
    c22 = _msub(az(3, m3), m2)
    m5 = g(5)
    c11 = _msub(az(0, m4), m5)
    c12 = _madd(az(1, m3), m5)
    m1 = g(1)
    c22 = _madd(c22, m1)
    c11 = _madd(c11, m1)
    c22 = _madd(c22, g(6))
    c11 = _madd(c11, g(7))
    return [r + s for r, s in zip(c11, c12)] + [r + s for r, s in zip(c21, c22)]


def _prep_weights(level, tile, a, az, rows):
    g = 2 ** level
    kt = 4 // g
    lo = lax.broadcasted_iota(jnp.int32, (16, 128), 1) < 64

    def shared(x, ty, k):
        if k < 3:
            return tile(2 * x + ty, k)
        if ty == 0:
            return jnp.where(lo, tile(2 * x, 3), tile(2 * x, 3) - tile(2 * x + 1, 3))
        return jnp.where(lo, tile(2 * x + 1, 3), tile(2 * x + 1, 4) - tile(2 * x, 4))

    for x in range(g):
        az[x, rows, :] = jnp.where(lo, tile(2 * x + 1, 4), tile(2 * x, 4)).astype(bf16)
    for ty in range(2):
        for k in range(kt):
            blocks = [[shared(x, ty, kb * kt + k) for kb in range(g)] for x in range(g)]
            for p, s in enumerate(_a_sums(blocks)):
                a[ty, p, k, rows, :] = s.astype(bf16)


def _prep_acts(level, x):
    g = 2 ** level
    kg, tw = 512 // g, TB // g

    def sums(starts, n):
        return [s.astype(bf16) for s in
                _b_sums([[x[r:r + n, tw * t:tw * (t + 1)] for t in range(g)] for r in starts])]

    head = sums([kg * kb for kb in range(g)], kg - 64)
    tails = [sums([kg * (kb + 1) - 64 for kb in range(g - 1)] + [last], 64) for last in (448, 512)]
    return [[jnp.concatenate([a, b], axis=0) for a, b in zip(head, tail)] for tail in tails], x[448:576].astype(bf16)


def _matmul(level, a, az, row, n, rhs, tick=lambda: None):
    g = 2 ** level
    tw = TB // g
    b, bz = rhs
    zs = [_dot(_load_bf16(az, (x,), row, n), bz) for x in range(g)]
    zs = [[z[:, tw * t:tw * (t + 1)] for t in range(g)] for z in zs]
    cs = []
    for ty in range(2):
        def product(p):
            tick()
            return _dot(_load_wide(a, (ty, p), row, n), b[ty][p])
        cs.append(_c_sums(product, 0, 7 ** level, zs))
    return [jnp.concatenate(cs[ty][x], axis=1) for x in range(g) for ty in range(2)]


def _kernel(x_hbm, wqkv_hbm, wo_hbm, wg_hbm, wu_hbm, wd_hbm, out_hbm,
            xio, wqkv, wo, wgu, wd, sems, slab, xslab, pipe0, pipe1, stage,
            aa, aza, agu, azgu, ad, xs, work):
    na = D // 2 ** (LA + 1)
    ng = UNIT // 2 ** (LG + 1)
    gd = 2 ** LD
    pipe = (pipe0, pipe1)
    nd, kd, td = D // gd, UNIT // gd, TB // gd

    def at(base, row, n, align=8):
        if isinstance(base, int):
            return pl.ds(base + row, n)
        return pl.ds(pl.multiple_of(base, align) + row, n)

    def tile_start(k):
        return jnp.minimum(k * 128, KT[-1])

    def half_copy(src, dst, first_sem, j):
        rows = at(j * 64, 0, 64, 64)
        return pltpu.make_async_copy(src.at[rows, :], dst.at[rows, :], sems.at[first_sem + j])

    def in_copies(j):
        return half_copy(wqkv_hbm, wqkv, 0, j), half_copy(x_hbm, xio, NH, j)

    cp_o = pltpu.make_async_copy(wo_hbm, wo, sems.at[2 * NH])
    cp_ffn = [pltpu.make_async_copy(wg_hbm, wgu.at[0], sems.at[2 * NH + 1]),
              pltpu.make_async_copy(wu_hbm, wgu.at[1], sems.at[2 * NH + 2]),
              pltpu.make_async_copy(wd_hbm, wd, sems.at[2 * NH + 3])]
    for j in range(AHEAD):
        for cp in in_copies(j):
            cp.start()

    def wt(s, k, row, n):
        return at((s * 5 + k) * D, QKV0 + row, n)

    @pl.loop(0, 5)
    def _(k):
        @pl.loop(2 * k, jnp.minimum(2 * k + 2, NH))
        def _(j):
            for cp in in_copies(j):
                cp.wait()

            @pl.when(j + AHEAD < NH)
            def _():
                for cp in in_copies(j + AHEAD):
                    cp.start()

            @pl.when(j == max(NH - AHEAD, 0))
            def _():
                cp_o.start()

        r0 = tile_start(k)
        xslab[...] = pltpu.bitcast(xio[at(r0, 0, 128, 64), :].T, u32)
        slab[0:3 * D // 2, :] = pltpu.bitcast(wqkv[at(r0, 0, 128, 64), :].T, u32)
        for c in range(NCOL):
            w2 = xslab[pl.ds(c, 128, stride=NCOL), :].T
            xs[at(r0, X0 + c * D, 128), :] = _unpack_lo(w2)
            xs[at(r0, X0 + (NCOL + c) * D, 128), :] = _unpack_hi(w2)
        for s in range(3):
            for j in range(DH // 2):
                w2 = slab[pl.ds(s * (D // 2) + j, H, stride=DH // 2), :]
                work[wt(0, k, 5 * s * D + 64 * j, 32), :] = _unpack_lo(w2)
                work[wt(0, k, 5 * s * D + 64 * j + 32, 32), :] = _unpack_hi(w2)

    cp_o.wait()
    for cp in cp_ffn:
        cp.start()
    for n in range(5):
        wn = min(128, D - 128 * n)
        blk = pltpu.bitcast(wo[:, 128 * n:128 * n + wn], u32)
        if wn < 128:
            blk = jnp.concatenate([blk, blk], axis=1)
        slab[n * D // 2:(n + 1) * D // 2, :] = blk
        rows = []
        for j in range(DH // 2):
            w2 = slab[pl.ds(n * D // 2 + j, H, stride=DH // 2), :]
            rows += [_unpack_lo(w2), _unpack_hi(w2)]
        wp = jnp.concatenate(rows, axis=0)
        for k, r0 in enumerate(KT):
            work[wt(3, k, 128 * n, wn), :] = wp[r0:r0 + 128].T[0:wn]

    @pl.loop(0, 4)
    def _(s):
        for r in range(0, na, 16):
            _prep_weights(LA, lambda i, k: work[wt(s, 0, k * D + na * i + r, 16), :], aa, aza, at(s * na, r, 16, 16))

    def put_stats(which, c, mean, squares):
        row = STAT0 + which * BC * 16
        var = jnp.sum(squares, axis=0, keepdims=True) * (1.0 / D)
        if mean is not None:
            xs[at(c * 16, row, 8), :] = jnp.broadcast_to(mean, (8, 128))
        xs[at(c * 16, row + 8, 8), :] = jnp.broadcast_to(lax.rsqrt(var + 1e-5) * (0.5 if which else 1.0), (8, 128))

    def norm_stats(which, c, x):
        mean = jnp.sum(x, axis=0, keepdims=True) * (1.0 / D)
        xc = x - mean
        put_stats(which, c, mean, xc * xc)

    def norm_stats_serial(blk, which):
        base = blk * (BC * D)
        for c in range(BC):
            tot = xs[at(base, X0 + c * D, 8), :]
            for r in range(8, D, 8):
                tot = tot + xs[at(base, X0 + c * D + r, 8), :]
            mean = jnp.broadcast_to(jnp.sum(tot, axis=0, keepdims=True) * (1.0 / D), (8, 128))
            xs[at(c * 16, STAT0 + which * BC * 16, 8), :] = mean
            tot = None
            for r in range(0, D, 8):
                xc = xs[at(base, X0 + c * D + r, 8), :] - mean
                tot = xc * xc if tot is None else tot + xc * xc
            put_stats(which, c, None, tot)

    def normed(blk, which):
        base = blk * (BC * D)
        cols = []
        for c in range(BC):
            row = STAT0 + (which * BC + c) * 16
            x = xs[at(base, X0 + c * D, D), :].reshape(D // 8, 8, 128)
            cols.append(((x - xs[row:row + 8, :]) * xs[row + 8:row + 16, :]).reshape(D, 128))
        return jnp.concatenate(cols, axis=1)

    def qkv_base(blk):
        return ((blk // 2) * (5 * NCOL) + (blk % 2) * BC) * D

    def qkv_proj(blk):
        base = qkv_base(blk)
        out = _matmul(LA, aa, aza, 0, 3 * na, _prep_acts(LA, normed(blk, 0)))
        for i, o in enumerate(out):
            for c in range(BC):
                oc = o[:, 128 * c:128 * (c + 1)]
                row = QKV0 + c * D + na * i
                work[at(base, row, na), :] = oc[0:na]
                for s in (1, 2):
                    val = oc[s * na:(s + 1) * na]
                    work[at(base, row + 2 * s * NCOL * D, na), :] = val
                    work[at(base, row + (2 * s - 1) * NCOL * D, na), :] = pltpu.roll(val, 1, 1)

    def softmax(logit, first_col, cols):
        pos = lax.broadcasted_iota(jnp.int32, (8, 128), 1) * NCOL + first_col
        logit = [l if w <= cols else jnp.where(pos >= w - cols, l, -1e9) for w, l in enumerate(logit)]
        top = logit[0]
        for l in logit[1:]:
            top = jnp.maximum(top, l)
        e = [jnp.exp(l - top) for l in logit]
        den = e[0]
        for x in e[1:]:
            den = den + x
        inv = 1.0 / den
        return [x * inv for x in e]

    def attend_serial(blk):
        base = qkv_base(blk)
        nc = ANC
        for c0 in range(0, BC, nc):
            for h in range(0, H, 8):
                row = QKV0 + c0 * D + h
                q = [[work[at(base, row + c * D + H * d, 8), :] for d in range(DH)] for c in range(nc)]
                for j in range(1 - W, nc):
                    cols = [c for c in range(nc) if 0 <= c - j < W]
                    acc = {}
                    for d in range(DH):
                        k = work[at(base, row + (2 * NCOL + j) * D + H * d, 8), :]
                        for c in cols:
                            acc[c] = q[c][d] * k if d == 0 else acc[c] + q[c][d] * k
                    for c in cols:
                        work[at(P0, 8 * (c * W + c - j), 8), :] = acc[c] * (DH ** -0.5)
                p = [softmax([work[at(P0, 8 * (c * W + w), 8), :] for w in range(W)], (blk % 2) * BC, c0 + c)
                     for c in range(nc)]
                for d in range(DH):
                    acc = {}
                    for j in range(1 - W, nc):
                        v = work[at(base, row + (4 * NCOL + j) * D + H * d, 8), :]
                        for c in range(nc):
                            if 0 <= c - j < W:
                                acc[c] = p[c][c - j] * v if c not in acc else acc[c] + p[c][c - j] * v
                    for c in range(nc):
                        work[at(O0, (c0 + c) * D + H * d + h, 8), :] = acc[c]

    def attend_first():
        nc = 2

        @pl.loop(0, (BC // nc) * (H // 8))
        def _(n):
            c0 = (n // (H // 8)) * nc
            base = c0 * D + (n % (H // 8)) * 8
            logit = [[None] * W for _ in range(nc)]
            for d in range(DH):
                k = {j: work[at(base, QKV0 + (2 * NCOL + j) * D + H * d, 8), :] for j in range(1 - W, nc)}
                for c in range(nc):
                    q = work[at(base, QKV0 + c * D + H * d, 8), :]
                    for w in range(W):
                        term = q * k[c - w]
                        logit[c][w] = term if d == 0 else logit[c][w] + term
            p = [softmax([l * (DH ** -0.5) for l in logit[c]], c0, c) for c in range(nc)]
            for d in range(DH):
                v = {j: work[at(base, QKV0 + (4 * NCOL + j) * D + H * d, 8), :] for j in range(1 - W, nc)}
                for c in range(nc):
                    acc = None
                    for w in range(W):
                        term = p[c][w] * v[c - w]
                        acc = term if w == 0 else acc + term
                    work[at(base, O0 + c * D + H * d, 8), :] = acc

    def out_proj(blk):
        base = blk * (BC * D)
        o = jnp.concatenate([work[at(O0, c * D, D), :] for c in range(BC)], axis=1)
        y = jnp.concatenate(_matmul(LA, aa, aza, 3 * na, na, _prep_acts(LA, o)), axis=0)
        x = [xs[at(base, X0 + c * D, D), :] + y[:, 128 * c:128 * (c + 1)] for c in range(BC)]
        for c in range(BC):
            xs[at(base, X0 + c * D, D), :] = x[c]
        for c in range(BC):
            norm_stats(1, c, x[c])

    def prep_ffn_weights():
        units = F // UNIT
        cp_ffn[0].wait()
        cp_ffn[1].wait()

        pipe[1][...] = jnp.zeros(pipe[1].shape, u32)

        @pl.loop(0, 2 * units + 1)
        def _(n):
            for slot in range(2):
                @pl.when(n % 2 == slot)
                def _():
                    cols = pl.ds(pl.multiple_of(jnp.minimum(n // 2, units - 1) * UNIT, UNIT), UNIT)
                    for k, r0 in enumerate(KT):
                        pipe[slot][k] = pltpu.bitcast(wgu[slot, r0:r0 + 128, cols].T, u32)
                    for r in range(0, ng, 16):
                        def tile(i, k):
                            return pltpu.bitcast(pipe[1 - slot][k, at(0, (i * ng + r) // 2, 8), :], bf16).astype(f32)
                        first = (jnp.maximum(n - 1, 0) // 2) * (2 * ng)
                        _prep_weights(LG, tile, agu, azgu, at(first, 2 * r + 16 * (1 - slot), 16, 16))

        cp_ffn[2].wait()

        @pl.loop(0, nd // 16)
        def _(r):
            for u in range(units):
                for k in range(0, kd, 128):
                    blocks = [[wd[at(16 * r, nd * x, 16, 16), pl.ds(u * UNIT + kd * kb + k, 128)].astype(f32)
                               for kb in range(gd)] for x in range(gd)]
                    for p, s in enumerate(_a_sums(blocks)):
                        ad[p, (u * kd + k) // 128, at(16 * r, 0, 16, 16), :] = s.astype(bf16)

    def ffn(i):
        blk = i % NBLK
        rhs = _prep_acts(LG, normed(blk, 1))
        n = F // UNIT * ng // NG
        hv = []
        for j in range(NG):
            gu = _matmul(LG, agu, azgu, 2 * n * j, 2 * n, rhs)
            gu = [t.reshape(n // 16, 2, 16, TB) for t in gu]
            hv.append([(t[:, 1] + t[:, 1] * jnp.tanh(t[:, 0])).reshape(n, TB) for t in gu])
        j, r, c = A_STAT
        xs[STAT0:STAT0 + 8, :] = hv[j][r][0:8, 128 * c:128 * (c + 1)]
        norm_stats_serial((i + 3) % NBLK, 0)
        j, r, c = A_ATT
        work[P0:P0 + 8, :] = hv[j][r][0:8, 128 * c:128 * (c + 1)]
        attend_serial((i + 1) % NBLK)
        piece = [jnp.concatenate([hv[j][r] for j in range(NG)], axis=0) for r in range(UNIT // ng)]
        h = [jnp.concatenate([t[ng * j:ng * (j + 1)] for t in piece], axis=0) for j in range(F // UNIT)]
        h = [jnp.concatenate([t[kd * a:kd * (a + 1)] for t in h], axis=0) for a in range(gd)]
        history = [hv[-1][r][0:8, 0:128] for r in HIST]
        sums = {(): [[t[:, td * c:td * (c + 1)] for c in range(gd)] for t in h]}

        def late(m, src):
            zero = jnp.tile(jnp.minimum(jnp.abs(src), 0.0), (1, td // 128))
            return [[(t.reshape(-1, 8, td) + zero).reshape(t.shape) for t in row] for row in m]

        if MODE[0] == "s":
            sums[()] = late(sums[()], history[0])

        def operand(path):
            if path not in sums:
                b11, b12, b21, b22 = _quad(operand(path[:-1]))
                op, first, *rest = ((_madd, b11, b22), (None, b11), (_msub, b12, b22), (_msub, b21, b11), (None, b22),
                                    (_madd, b11, b12), (_madd, b21, b22))[path[-1]]
                if MODE[len(path) - 1] == "z":
                    first = late(first, history[-len(HIST)])
                sums[path] = first if op is None else op(first, *rest)
            return sums[path]

        def down(p):
            rhs = operand(tuple(p // 7 ** (LD - 1 - l) % 7 for l in range(LD)))[0][0]
            prod = _dot(_load_wide(ad, (p,), 0, nd), rhs.astype(bf16))
            history.append(prod[0:8, 0:128])
            return prod

        y = _c_sums(down, 0, 7 ** LD)
        for x, row in enumerate(y):
            row = jnp.concatenate(row, axis=1)
            for c in range(BC):
                xs[at(blk * (BC * D), X0 + c * D + nd * x, nd), :] += row[:, 128 * c:128 * (c + 1)]

    @pl.loop(0, 2 * NBLK + 3)
    def _(n):
        @pl.when(n < 3)
        def _():
            x = [xs[at(n * BC * D, X0 + c * D, D), :] for c in range(BC)]
            for c in range(BC):
                norm_stats(0, c, x[c])

        @pl.when(n == 2)
        def _():
            attend_first()

        @pl.when(n == 3)
        def _():
            prep_ffn_weights()

        @pl.when(n >= 3)
        def _():
            ffn(n - 3)

        @pl.when((n >= 2) & (n < 2 * NBLK + 2))
        def _():
            out_proj((n - 2) % NBLK)

        @pl.when(n < 2 * NBLK)
        def _():
            qkv_proj(n % NBLK)

    @pl.loop(0, 5)
    def _(k):
        r0 = D - 128 - tile_start(k)
        for c in range(NCOL):
            pair = pltpu.pack_elementwise([xs[at(r0, X0 + c * D, 128), :],
                                           xs[at(r0, X0 + (NCOL + c) * D, 128), :]], packed_dtype=bf16)
            xslab[pl.ds(c, 128, stride=NCOL), :] = pltpu.bitcast(pair, u32).T
        stage[k] = pltpu.bitcast(xslab[...], bf16).T
        pltpu.make_async_copy(stage.at[k, 0:64], out_hbm.at[at(r0, 0, 64, 64), :], sems.at[0]).start()

        @pl.when(k < 4)
        def _():
            pltpu.make_async_copy(stage.at[k, 64:128], out_hbm.at[at(r0, 64, 64, 64), :], sems.at[0]).start()

    pltpu.make_async_copy(xio, out_hbm, sems.at[0]).wait()


def _weight_scratch(level, rows):
    g = 2 ** level
    return [pltpu.VMEM((2, 7 ** level, 4 // g, rows // (2 * g), 128), bf16),
            pltpu.VMEM((g, rows // (2 * g), 128), bf16)]


@jax.jit
def pallas_interleave_layers__sliding_local_dilated__glu_gated_glu__prompt_kernel(
        A_x, A_wqkv, A_wo, B_x, B_w_gate, B_w_up, B_w_down):
    del B_x
    any_spec = pl.BlockSpec(memory_space=pl.ANY)
    V = pltpu.VMEM
    out = pl.pallas_call(
        _kernel,
        out_shape=jax.ShapeDtypeStruct((D, S), bf16),
        in_specs=[any_spec] * 6,
        out_specs=any_spec,
        scratch_shapes=[
            V((D, S), bf16), V((D, 3 * D), bf16), V((D, D), bf16),
            V((2, D, F), bf16), V((D, F), bf16),
            pltpu.SemaphoreType.DMA((2 * NH + 4,)),
            V((5 * D // 2, 128), u32), V((S // 2, 128), u32), V((5, UNIT // 2, 128), u32), V((5, UNIT // 2, 128), u32),
            V((5, 128, S), bf16),
            *_weight_scratch(LA, 4 * D), *_weight_scratch(LG, 2 * F),
            V((7 ** LD, F // 2 ** LD // 128, D // 2 ** LD, 128), bf16),
            V((X_ROWS, 128), f32), V((WORK_ROWS, 128), f32),
        ],
        compiler_params=pltpu.CompilerParams(vmem_limit_bytes=127 * 2**20),
    )(A_x[0].T, A_wqkv, A_wo, B_w_gate, B_w_up, B_w_down.T)
    return out.T[None]
```

```python
import math

import jax
import jax.numpy as jnp
from jax import lax
import jax.experimental.pallas as pl
import jax.experimental.pallas.tpu as pltpu

S, D, F = 2048, 576, 4608
H, DH, W = 32, 18, 8
NCOL = 8
BC = 4
TB = 128 * BC
NBLK = S // TB
KT = (0, 128, 256, 384, 448)
UNIT = 512
NH = D // 64
AHEAD = 4
UNROLL = 2
LA, LG, LD = 1, 2, 2
CHUNKS = (8, 4, 4, 4, 4, 4, 4, 4)
A_STAT = (6, 1, 0)
A_ATT = (1, 1, 0)
ORD_G = ('2435167r', '2435167')
ORD_D = ('2435167', '2514376')
ORD_Q = ('2543167r',)
ORD_O = ("2435167",)
ANC = 1
QREL = 0
FNC = 4
FUN = None
HIST = (5, 5, 5)
MODE = '-z'

f32 = jnp.float32
bf16 = jnp.bfloat16
u32 = jnp.uint32

X0 = 0
XB = BC * (D + 16)
STAT0 = X0 + BC * D
X_ROWS = NBLK * XB
QKV0 = 0
O0 = QKV0 + 2 * 5 * NCOL * D
P0 = O0 + BC * D
WORK_ROWS = P0 + BC * W * 8


def _dot(a, b):
    return jnp.dot(a, b, preferred_element_type=f32)


def _unpack_lo(w):
    return pltpu.bitcast(w << 16, f32)


def _unpack_hi(w):
    return pltpu.bitcast(w & u32(0xFFFF0000), f32)


def _load_bf16(ref, idx, row, n):
    return pltpu.bitcast(ref.bitcast(u32)[(*idx, slice(row // 2, (row + n) // 2))], bf16)


def _load_wide(ref, idx, row, n):
    return jnp.concatenate([_load_bf16(ref, (*idx, k), row, n) for k in range(ref.shape[len(idx)])], axis=1)


def _madd(a, b):
    return [[x + y for x, y in zip(r, s)] for r, s in zip(a, b)]


def _msub(a, b):
    return [[x - y for x, y in zip(r, s)] for r, s in zip(a, b)]


def _quad(m):
    n = len(m) // 2
    return ([r[:n] for r in m[:n]], [r[n:] for r in m[:n]], [r[:n] for r in m[n:]], [r[n:] for r in m[n:]])


def _a_sums(m):
    if len(m) == 1:
        yield m[0][0]
        return
    a11, a12, a21, a22 = _quad(m)
    yield from _a_sums(_madd(a11, a22))
    yield from _a_sums(_madd(a21, a22))
    yield from _a_sums(a11)
    yield from _a_sums(a22)
    yield from _a_sums(_madd(a11, a12))
    yield from _a_sums(_msub(a21, a11))
    yield from _a_sums(_msub(a12, a22))


def _b_sums(m):
    if len(m) == 1:
        yield m[0][0]
        return
    b11, b12, b21, b22 = _quad(m)
    yield from _b_sums(_madd(b11, b22))
    yield from _b_sums(b11)
    yield from _b_sums(_msub(b12, b22))
    yield from _b_sums(_msub(b21, b11))
    yield from _b_sums(b22)
    yield from _b_sums(_madd(b11, b12))
    yield from _b_sums(_madd(b21, b22))


C_TERMS = ({1: 1, 4: 1, 5: -1, 7: 1}, {3: 1, 5: 1}, {2: 1, 4: 1}, {1: 1, 2: -1, 3: 1, 6: 1})


def _c_sums(product, first, orders, z=None):
    if not orders:
        m = product(first)
        return [[m if z is None else m + z[0][0]]]
    k = 7 ** (len(orders) - 1)
    order, tree = orders[0][:7], orders[0][7:]
    m = {int(i): _c_sums(product, first + (int(i) - 1) * k, orders[1:]) for i in order}
    out = []
    for q, terms in enumerate(C_TERMS):
        vals = [(terms[i], v) for i, v in m.items() if i in terms]
        if z is not None:
            vals.insert(len(vals) if "l" in tree else 0, (1, _quad(z)[q]))
        if "r" in tree:
            vals.reverse()
        sign, acc = vals[0]
        for sg, v in vals[1:]:
            acc = _madd(acc, v) if sg == sign else _msub(acc, v) if sign == 1 else _msub(v, acc)
            sign = 1
        out.append(acc)
    c11, c12, c21, c22 = out
    return [r + s for r, s in zip(c11, c12)] + [r + s for r, s in zip(c21, c22)]


def _prep_weights(level, tile, a, az, rows, tick=lambda: None):
    g = 2 ** level
    kt = 4 // g
    lo = lax.broadcasted_iota(jnp.int32, (16, 128), 1) < 64

    def shared(x, ty, k):
        if k < 3:
            return tile(2 * x + ty, k)
        if ty == 0:
            return jnp.where(lo, tile(2 * x, 3), tile(2 * x, 3) - tile(2 * x + 1, 3))
        return jnp.where(lo, tile(2 * x + 1, 3), tile(2 * x + 1, 4) - tile(2 * x, 4))

    for x in range(g):
        az[x, rows, :] = jnp.where(lo, tile(2 * x + 1, 4), tile(2 * x, 4)).astype(bf16)
    for ty in range(2):
        for k in range(kt):
            blocks = [[shared(x, ty, kb * kt + k) for kb in range(g)] for x in range(g)]
            for p, s in enumerate(_a_sums(blocks)):
                a[ty, p, k, rows, :] = s.astype(bf16)
        tick()


def _prep_acts(level, x):
    g = 2 ** level
    kg, tw = 512 // g, TB // g

    def sums(starts, n):
        return [s.astype(bf16) for s in
                _b_sums([[x[r:r + n, tw * t:tw * (t + 1)] for t in range(g)] for r in starts])]

    head = sums([kg * kb for kb in range(g)], kg - 64)
    tails = [sums([kg * (kb + 1) - 64 for kb in range(g - 1)] + [last], 64) for last in (448, 512)]
    return [[jnp.concatenate([a, b], axis=0) for a, b in zip(head, tail)] for tail in tails], x[448:576].astype(bf16)


def _matmul(level, a, az, row, n, rhs, orders):
    g = 2 ** level
    tw = TB // g
    b, bz = rhs
    zs = [_dot(_load_bf16(az, (x,), row, n), bz) for x in range(g)]
    zs = [[z[:, tw * t:tw * (t + 1)] for t in range(g)] for z in zs]
    cs = []
    for ty in range(2):
        def product(p):
            return _dot(_load_wide(a, (ty, p), row, n), b[ty][p])
        cs.append(_c_sums(product, 0, orders, zs))
    return [jnp.concatenate(cs[ty][x], axis=1) for x in range(g) for ty in range(2)]


def _kernel(x_hbm, wqkv_hbm, wo_hbm, wg_hbm, wu_hbm, wd_hbm, out_hbm,
            xio, wqkv, wo, wgu, wd, sems, slab, xslab, stage,
            aa, aza, agu, azgu, ad, xs, work):
    na = D // 2 ** (LA + 1)
    ng = 128 // 2 ** (LG + 1)

    def piece_row(i):
        return (i % 2) * 64 + (i // 2) * ng

    gd = 2 ** LD
    nd, kd, td = D // gd, UNIT // gd, TB // gd

    def at(base, row, n, align=8):
        if isinstance(base, int):
            return pl.ds(base + row, n)
        return pl.ds(pl.multiple_of(base, align) + row, n)

    def tile_start(k):
        return jnp.minimum(k * 128, KT[-1])

    def half_copy(src, dst, first_sem, j):
        rows = at(j * 64, 0, 64, 64)
        return pltpu.make_async_copy(src.at[rows, :], dst.at[rows, :], sems.at[first_sem + j])

    def in_copies(j):
        return half_copy(wqkv_hbm, wqkv, 0, j), half_copy(x_hbm, xio, NH, j)

    cp_o = pltpu.make_async_copy(wo_hbm, wo, sems.at[2 * NH])
    cp_ffn = [pltpu.make_async_copy(wg_hbm, wgu.at[0], sems.at[2 * NH + 1]),
              pltpu.make_async_copy(wu_hbm, wgu.at[1], sems.at[2 * NH + 2]),
              pltpu.make_async_copy(wd_hbm, wd, sems.at[2 * NH + 3])]
    for j in range(AHEAD):
        for cp in in_copies(j):
            cp.start()

    def wt(s, k, row, n):
        return at((s * 5 + k) * D, QKV0 + row, n)

    @pl.loop(0, 5)
    def _(k):
        @pl.loop(2 * k, jnp.minimum(2 * k + 2, NH))
        def _(j):
            for cp in in_copies(j):
                cp.wait()

            @pl.when(j + AHEAD < NH)
            def _():
                for cp in in_copies(j + AHEAD):
                    cp.start()

            @pl.when(j == max(NH - AHEAD, 0))
            def _():
                cp_o.start()

        r0 = tile_start(k)
        xslab[...] = pltpu.bitcast(xio[at(r0, 0, 128, 64), :].T, u32)
        slab[0:3 * D // 2, :] = pltpu.bitcast(wqkv[at(r0, 0, 128, 64), :].T, u32)
        for c in range(NCOL):
            w2 = xslab[pl.ds(c, 128, stride=NCOL), :].T
            xs[at(r0, X0 + c // BC * XB + c % BC * D, 128), :] = _unpack_lo(w2)
            xs[at(r0, X0 + (2 + c // BC) * XB + c % BC * D, 128), :] = _unpack_hi(w2)
        for s in range(3):
            for j in range(DH // 2):
                w2 = slab[pl.ds(s * (D // 2) + j, H, stride=DH // 2), :]
                work[wt(0, k, 5 * s * D + 64 * j, 32), :] = _unpack_lo(w2)
                work[wt(0, k, 5 * s * D + 64 * j + 32, 32), :] = _unpack_hi(w2)

    cp_o.wait()
    for cp in cp_ffn:
        cp.start()
    for n in range(5):
        wn = min(128, D - 128 * n)
        blk = pltpu.bitcast(wo[:, 128 * n:128 * n + wn], u32)
        if wn < 128:
            blk = jnp.concatenate([blk, blk], axis=1)
        slab[n * D // 2:(n + 1) * D // 2, :] = blk
        rows = []
        for j in range(DH // 2):
            w2 = slab[pl.ds(n * D // 2 + j, H, stride=DH // 2), :]
            rows += [_unpack_lo(w2), _unpack_hi(w2)]
        wp = jnp.concatenate(rows, axis=0)
        for k, r0 in enumerate(KT):
            work[wt(3, k, 128 * n, wn), :] = wp[r0:r0 + 128].T[0:wn]

    @pl.loop(0, 4)
    def _(s):
        for r in range(0, na, 16):
            _prep_weights(LA, lambda i, k: work[wt(s, 0, k * D + na * i + r, 16), :], aa, aza, at(s * na, r, 16, 16))

    def mean_of(tot):
        return jnp.broadcast_to(jnp.sum(tot, axis=0, keepdims=True) * (1.0 / D), (8, 128))

    def norm_stats(blk, serial):
        base = blk * XB
        groups = [[c] for c in range(BC)] if serial else [range(BC)]
        for cols in groups:
            mean = {}
            for c in cols:
                tot = xs[at(base, X0 + c * D, 8), :]
                for r in range(8, D, 8):
                    tot = tot + xs[at(base, X0 + c * D + r, 8), :]
                mean[c] = mean_of(tot)
                xs[at(base, STAT0 + 16 * c, 8), :] = mean[c]
            if serial:
                xs[X_ROWS:X_ROWS + 8, :] = mean[c]
            for c in cols:
                tot = None
                for r in range(0, D, 8):
                    xc = xs[at(base, X0 + c * D + r, 8), :] - mean[c]
                    tot = xc * xc if tot is None else tot + xc * xc
                rstd = lax.rsqrt(mean_of(tot) + 1e-5)
                xs[at(base, STAT0 + 16 * c + 8, 8), :] = rstd
            if serial:
                xs[X_ROWS:X_ROWS + 8, :] = rstd

    def normed(blk, scale):
        base = blk * XB
        cols = []
        for c in range(BC):
            x = xs[at(base, X0 + c * D, D), :].reshape(D // 8, 8, 128)
            mean, rstd = xs[at(base, STAT0 + 16 * c, 8), :], xs[at(base, STAT0 + 16 * c + 8, 8), :]
            cols.append(((x - mean) * (rstd * scale)).reshape(D, 128))
        return jnp.concatenate(cols, axis=1)

    def qkv_base(blk):
        return ((blk // 2) * (5 * NCOL) + (blk % 2) * BC) * D

    def qkv_proj(blk, stats_blk):
        base = qkv_base(blk)
        out = _matmul(LA, aa, aza, 0, 3 * na, _prep_acts(LA, normed(blk, 1.0)), ORD_Q)
        norm_stats(stats_blk, True)
        for i, o in enumerate(out):
            for c in range(BC):
                oc = o[:, 128 * c:128 * (c + 1)]
                row = QKV0 + c * D + na * i
                work[at(base, row, na), :] = oc[0:na]
                for s in (1, 2):
                    val = oc[s * na:(s + 1) * na]
                    work[at(base, row + 2 * s * NCOL * D, na), :] = val
                    work[at(base, row + (2 * s - 1) * NCOL * D, na), :] = pltpu.roll(val, 1, 1)

    def softmax(logit, first_col, cols):
        pos = lax.broadcasted_iota(jnp.int32, (8, 128), 1) * NCOL + first_col
        logit = [l if w <= cols else jnp.where(pos >= w - cols, l, -1e9) for w, l in enumerate(logit)]
        top = logit[0]
        for l in logit[1:]:
            top = jnp.maximum(top, l)
        e = [jnp.exp(l - top) for l in logit]
        den = e[0]
        for x in e[1:]:
            den = den + x
        inv = 1.0 / den
        return [x * inv for x in e]

    def attend_serial(blk):
        base = qkv_base(blk)
        nc = ANC
        for c0 in range(0, BC, nc):
            for h in range(0, H, 8):
                row = QKV0 + c0 * D + h
                q = [[work[at(base, row + c * D + H * d, 8), :] for d in range(DH)] for c in range(nc)]
                for j in range(1 - W, nc):
                    cols = [c for c in range(nc) if 0 <= c - j < W]
                    acc = {}
                    if QREL:
                        q = [[work[at(base, row + c * D + H * d, 8), :] for d in range(DH)] for c in range(nc)]
                    for d in range(DH):
                        k = work[at(base, row + (2 * NCOL + j) * D + H * d, 8), :]
                        for c in cols:
                            acc[c] = q[c][d] * k if d == 0 else acc[c] + q[c][d] * k
                    for c in cols:
                        work[at(P0, 8 * (c * W + c - j), 8), :] = acc[c] * (DH ** -0.5)
                p = [softmax([work[at(P0, 8 * (c * W + w), 8), :] for w in range(W)], (blk % 2) * BC, c0 + c)
                     for c in range(nc)]
                for d in range(DH):
                    acc = {}
                    for j in range(1 - W, nc):
                        v = work[at(base, row + (4 * NCOL + j) * D + H * d, 8), :]
                        for c in range(nc):
                            if 0 <= c - j < W:
                                acc[c] = p[c][c - j] * v if c not in acc else acc[c] + p[c][c - j] * v
                    for c in range(nc):
                        work[at(O0, (c0 + c) * D + H * d + h, 8), :] = acc[c]

    def attend_first():
        nc = FNC

        @pl.loop(0, (BC // nc) * (H // 8), unroll=FUN)
        def _(n):
            c0 = (n // (H // 8)) * nc
            base = c0 * D + (n % (H // 8)) * 8
            logit = [[None] * W for _ in range(nc)]
            for d in range(DH):
                k = {j: work[at(base, QKV0 + (2 * NCOL + j) * D + H * d, 8), :] for j in range(1 - W, nc)}
                for c in range(nc):
                    q = work[at(base, QKV0 + c * D + H * d, 8), :]
                    for w in range(W):
                        term = q * k[c - w]
                        logit[c][w] = term if d == 0 else logit[c][w] + term
            p = [softmax([l * (DH ** -0.5) for l in logit[c]], c0, c) for c in range(nc)]
            for d in range(DH):
                v = {j: work[at(base, QKV0 + (4 * NCOL + j) * D + H * d, 8), :] for j in range(1 - W, nc)}
                for c in range(nc):
                    acc = None
                    for w in range(W):
                        term = p[c][w] * v[c - w]
                        acc = term if w == 0 else acc + term
                    work[at(base, O0 + c * D + H * d, 8), :] = acc

    def out_proj(blk):
        base = blk * XB
        o = jnp.concatenate([work[at(O0, c * D, D), :] for c in range(BC)], axis=1)
        y = jnp.concatenate(_matmul(LA, aa, aza, 3 * na, na, _prep_acts(LA, o), ORD_O), axis=0)
        for c in range(BC):
            xs[at(base, X0 + c * D, D), :] += y[:, 128 * c:128 * (c + 1)]

    def prep_ffn_weights():
        units = F // UNIT
        cp_ffn[0].wait()
        cp_ffn[1].wait()

        @pl.loop(0, F // 128 // UNROLL)
        def _(n):
            for t in range(UNROLL):
                for which in range(2):
                    col = pl.ds(pl.multiple_of(n * UNROLL * 128, 128) + t * 128, 128)
                    src = [wgu[which, r0:r0 + 128, col].T.astype(f32) for r0 in KT]
                    for r in range(0, ng, 16):
                        _prep_weights(LG, lambda i, k: src[k][piece_row(i) + r:piece_row(i) + r + 16], agu, azgu,
                                      at(n * UNROLL * 2 * ng, 2 * (t * ng + r) + 16 * which, 16, 16))

        cp_ffn[2].wait()

        @pl.loop(0, nd // 16)
        def _(r):
            for u in range(units):
                for k in range(0, kd, 128):
                    blocks = [[wd[at(16 * r, nd * x, 16, 16), pl.ds(u * UNIT + kd * kb + k, 128)].astype(f32)
                               for kb in range(gd)] for x in range(gd)]
                    for p, s in enumerate(_a_sums(blocks)):
                        ad[p, (u * kd + k) // 128, at(16 * r, 0, 16, 16), :] = s.astype(bf16)

    def ffn(i):
        blk = i % NBLK
        rhs = _prep_acts(LG, normed(blk, 0.5))
        hv, row = [], 0
        for n in CHUNKS:
            gu = _matmul(LG, agu, azgu, 32 * row, 32 * n, rhs, ORD_G)
            gu = [t.reshape(n, 2, 16, TB) for t in gu]
            hv.append([(t[:, 1] + t[:, 1] * jnp.tanh(t[:, 0])).reshape(16 * n, TB) for t in gu])
            row += n
        j, r, c = A_STAT
        xs[X_ROWS:X_ROWS + 8, :] = hv[j][r][0:8, 128 * c:128 * (c + 1)]
        norm_stats((i + 3) % NBLK, True)
        j, r, c = A_ATT
        work[P0:P0 + 8, :] = hv[j][r][0:8, 128 * c:128 * (c + 1)]
        attend_serial((i + 1) % NBLK)
        piece = [jnp.concatenate([t[r] for t in hv], axis=0)
                 for r in sorted(range(128 // ng), key=piece_row)]
        h = [jnp.concatenate([t[ng * j:ng * (j + 1)] for j in range(F // 128) if j * 128 % UNIT // kd == a
                              for t in piece], axis=0) for a in range(gd)]
        history = [hv[-1][r][0:8, 0:128] for r in HIST]
        sums = {(): [[t[:, td * c:td * (c + 1)] for c in range(gd)] for t in h]}

        def late(m, src):
            zero = jnp.tile(jnp.minimum(jnp.abs(src), 0.0), (1, td // 128))
            return [[(t.reshape(-1, 8, td) + zero).reshape(t.shape) for t in row] for row in m]

        if MODE[0] == "s":
            sums[()] = late(sums[()], history[0])

        def operand(path):
            if path not in sums:
                b11, b12, b21, b22 = _quad(operand(path[:-1]))
                op, first, *rest = ((_madd, b11, b22), (None, b11), (_msub, b12, b22), (_msub, b21, b11), (None, b22),
                                    (_madd, b11, b12), (_madd, b21, b22))[path[-1]]
                if MODE[len(path) - 1] == "z":
                    first = late(first, history[-len(HIST)])
                sums[path] = first if op is None else op(first, *rest)
            return sums[path]

        def down(p):
            rhs = operand(tuple(p // 7 ** (LD - 1 - l) % 7 for l in range(LD)))[0][0]
            prod = _dot(_load_wide(ad, (p,), 0, nd), rhs.astype(bf16))
            history.append(prod[0:8, 0:128])
            return prod

        y = _c_sums(down, 0, ORD_D)
        for x, row in enumerate(y):
            row = jnp.concatenate(row, axis=1)
            for c in range(BC):
                xs[at(blk * XB, X0 + c * D + nd * x, nd), :] += row[:, 128 * c:128 * (c + 1)]

    @pl.loop(0, 2 * NBLK + 3)
    def _(n):
        @pl.when((n == 0) | (n > 2 * NBLK))
        def _():
            norm_stats(jnp.maximum(n - 3, 0) % NBLK, False)

        @pl.when(n == 2)
        def _():
            attend_first()

        @pl.when(n == 3)
        def _():
            prep_ffn_weights()

        @pl.when(n >= 3)
        def _():
            ffn(n - 3)

        @pl.when((n >= 2) & (n < 2 * NBLK + 2))
        def _():
            out_proj((n - 2) % NBLK)

        @pl.when(n < 2 * NBLK)
        def _():
            qkv_proj(n % NBLK, jnp.where(n < 2, n + 1, n - 2) % NBLK)

    @pl.loop(0, 5)
    def _(k):
        r0 = D - 128 - tile_start(k)
        for c in range(NCOL):
            pair = pltpu.pack_elementwise([xs[at(r0, X0 + c // BC * XB + c % BC * D, 128), :],
                                           xs[at(r0, X0 + (2 + c // BC) * XB + c % BC * D, 128), :]], packed_dtype=bf16)
            xslab[pl.ds(c, 128, stride=NCOL), :] = pltpu.bitcast(pair, u32).T
        stage[k] = pltpu.bitcast(xslab[...], bf16).T
        pltpu.make_async_copy(stage.at[k, 0:64], out_hbm.at[at(r0, 0, 64, 64), :], sems.at[0]).start()

        @pl.when(k < 4)
        def _():
            pltpu.make_async_copy(stage.at[k, 64:128], out_hbm.at[at(r0, 64, 64, 64), :], sems.at[0]).start()

    pltpu.make_async_copy(xio, out_hbm, sems.at[0]).wait()


def _weight_scratch(level, rows):
    g = 2 ** level
    return [pltpu.VMEM((2, 7 ** level, 4 // g, rows // (2 * g), 128), bf16),
            pltpu.VMEM((g, rows // (2 * g), 128), bf16)]


@jax.jit
def pallas_interleave_layers__sliding_local_dilated__glu_gated_glu__prompt_kernel(
        A_x, A_wqkv, A_wo, B_x, B_w_gate, B_w_up, B_w_down):
    del B_x
    any_spec = pl.BlockSpec(memory_space=pl.ANY)
    V = pltpu.VMEM
    out = pl.pallas_call(
        _kernel,
        out_shape=jax.ShapeDtypeStruct((D, S), bf16),
        in_specs=[any_spec] * 6,
        out_specs=any_spec,
        scratch_shapes=[
            V((D, S), bf16), V((D, 3 * D), bf16), V((D, D), bf16),
            V((2, D, F), bf16), V((D, F), bf16),
            pltpu.SemaphoreType.DMA((2 * NH + 4,)),
            V((5 * D // 2, 128), u32), V((S // 2, 128), u32),
            V((5, 128, S), bf16),
            *_weight_scratch(LA, 4 * D), *_weight_scratch(LG, 2 * F),
            V((7 ** LD, F // 2 ** LD // 128, D // 2 ** LD, 128), bf16),
            V((X_ROWS + 8, 128), f32), V((WORK_ROWS, 128), f32),
        ],
        compiler_params=pltpu.CompilerParams(vmem_limit_bytes=127 * 2**20),
    )(A_x[0].T, A_wqkv, A_wo, B_w_gate, B_w_up, B_w_down.T)
    return out.T[None]
```

```python
import jax
import jax.numpy as jnp
from jax import lax
import jax.experimental.pallas as pl
import jax.experimental.pallas.tpu as pltpu

S, D, F = 2048, 576, 4608
H, DH, W = 32, 18, 8
NCOL = 8
BC = 4
TB = 128 * BC
NBLK = S // TB
KT = (0, 128, 256, 384, 448)
NA = ND = D // 4
NH = D // 64

ORDER_QKV = ("2543167r",)
ORDER_OUT = ("2435167",)
ORDER_GATE_UP = ("2435167r", "2435167")
ORDER_DOWN = ("2435167", "2514376")
GATE_UP_CHUNKS = (8, 4, 4, 4, 4, 4, 4, 4)
PREP_UNROLL = 6
ATTEND_AFTER, STATS_AFTER = 0, 6

STAT0 = BC * D
XB = STAT0 + BC * 16
XPAD = NBLK * XB
O0 = 2 * 5 * NCOL * D
P0 = O0 + BC * D
PAD = P0 + BC * W * 8

f32 = jnp.float32
bf16 = jnp.bfloat16
u32 = jnp.uint32


def _dot(a, b):
    return jnp.dot(a, b, preferred_element_type=f32)


def _unpack_lo(w):
    return pltpu.bitcast(w << 16, f32)


def _unpack_hi(w):
    return pltpu.bitcast(w & u32(0xFFFF0000), f32)


def _bf16_bits(x):
    return pltpu.bitcast(x.astype(bf16).astype(f32), u32)


def _rows(base, row, n, align=8):
    if isinstance(base, int):
        return pl.ds(base + row, n)
    return pl.ds(pl.multiple_of(base, align) + row, n)


def _load(ref, idx, row, n):
    return pltpu.bitcast(ref.bitcast(u32)[(*idx, slice(row // 2, (row + n) // 2))], bf16)


def _load_wide(ref, idx, row, n):
    return jnp.concatenate([_load(ref, (*idx, k), row, n) for k in range(ref.shape[len(idx)])], axis=1)


def _madd(a, b):
    return [[x + y for x, y in zip(r, s)] for r, s in zip(a, b)]


def _msub(a, b):
    return [[x - y for x, y in zip(r, s)] for r, s in zip(a, b)]


def _first(a):
    return a


def _quad(m):
    n = len(m) // 2
    return ([r[:n] for r in m[:n]], [r[n:] for r in m[:n]], [r[:n] for r in m[n:]], [r[n:] for r in m[n:]])


A_TERMS = ((_madd, 0, 3), (_madd, 2, 3), (_first, 0), (_first, 3), (_madd, 0, 1), (_msub, 2, 0), (_msub, 1, 3))
B_TERMS = ((_madd, 0, 3), (_first, 0), (_msub, 1, 3), (_msub, 2, 0), (_first, 3), (_madd, 0, 1), (_madd, 2, 3))
C_TERMS = ({1: 1, 4: 1, 5: -1, 7: 1}, {3: 1, 5: 1}, {2: 1, 4: 1}, {1: 1, 2: -1, 3: 1, 6: 1})
MIRRORED = (2, 5, 6, 7)


def _operands(terms, m):
    if len(m) == 1:
        yield m[0][0]
        return
    quad = _quad(m)
    for op, *which in terms:
        yield from _operands(terms, op(*[quad[i] for i in which]))


def _combine(product, first, orders, addend=None, mirrored=()):
    if not orders:
        return [[product(first)]]
    order = [int(i) for i in orders[0][:7]]
    m = {i: _combine(product, first + (i - 1) * 7 ** (len(orders) - 1), orders[1:]) for i in order}
    for i in mirrored:
        m[i] = [row[::-1] for row in m[i]]
    out = []
    for q, terms in enumerate(C_TERMS):
        vals = [(terms[i], m[i]) for i in order if i in terms]
        if addend is not None:
            vals.insert(0, (1, _quad(addend)[q]))
        if orders[0].endswith("r"):
            vals.reverse()
        sign, acc = vals[0]
        for sg, v in vals[1:]:
            acc = _madd(acc, v) if sg == sign else _msub(acc, v) if sign == 1 else _msub(v, acc)
            sign = 1
        out.append(acc)
    return [r + s for r, s in zip(out[0], out[1])] + [r + s for r, s in zip(out[2], out[3])]


def _prep_weights(level, tile, a, az, rows):
    g = 2 ** level
    kt = 4 // g
    lo = lax.broadcasted_iota(jnp.int32, (16, 128), 1) < 64

    def own(x, ty, k):
        if k < 3:
            return tile(2 * x + ty, k)
        if ty == 0:
            return jnp.where(lo, tile(2 * x, 3), tile(2 * x, 3) - tile(2 * x + 1, 3))
        return jnp.where(lo, tile(2 * x + 1, 3), tile(2 * x + 1, 4) - tile(2 * x, 4))

    for x in range(g):
        az[x, rows, :] = jnp.where(lo, tile(2 * x + 1, 4), tile(2 * x, 4)).astype(bf16)
    for ty in range(2):
        for k in range(kt):
            blocks = [[own(x, ty, kb * kt + k) for kb in range(g)] for x in range(g)]
            for p, s in enumerate(_operands(A_TERMS, blocks)):
                a[ty, p, k, rows, :] = s.astype(bf16)


def _prep_acts(level, x):
    g = 2 ** level
    kg, tw = 512 // g, TB // g

    def sums(starts, n):
        blocks = [[x[r:r + n, tw * t:tw * (t + 1)] for t in range(g)] for r in starts]
        return [s.astype(bf16) for s in _operands(B_TERMS, blocks)]

    head = sums([kg * kb for kb in range(g)], kg - 64)
    tails = [sums([kg * (kb + 1) - 64 for kb in range(g - 1)] + [last], 64) for last in (448, 512)]
    return [[jnp.concatenate([a, b], axis=0) for a, b in zip(head, tail)] for tail in tails], x[448:576].astype(bf16)


def _matmul(a, az, row, n, rhs, orders):
    g = 2 ** len(orders)
    tw = TB // g
    b, bz = rhs
    shared = [_dot(_load(az, (x,), row, n), bz) for x in range(g)]
    shared = [[z[:, tw * t:tw * (t + 1)] for t in range(g)] for z in shared]
    out = [_combine(lambda p: _dot(_load_wide(a, (ty, p), row, n), b[ty][p]), 0, orders, shared) for ty in range(2)]
    return [jnp.concatenate(out[ty][x], axis=1) for x in range(g) for ty in range(2)]


def _softmax(logit, first_col, c):
    pos = lax.broadcasted_iota(jnp.int32, (8, 128), 1) * NCOL + first_col
    logit = [l if w <= c else jnp.where(pos >= w - c, l, -1e9) for w, l in enumerate(logit)]
    top = logit[0]
    for l in logit[1:]:
        top = jnp.maximum(top, l)
    e = [jnp.exp(l - top) for l in logit]
    den = e[0]
    for x in e[1:]:
        den = den + x
    inv = 1.0 / den
    return [x * inv for x in e]


def _kernel(x_hbm, wqkv_hbm, wo_hbm, wg_hbm, wu_hbm, wd_hbm, out_hbm,
            xin, wqkv, wo, wgu, wd, sems, slab, xslab, stage,
            aa, aaz, agu, aguz, ad, xs, att):

    def in_copies(j):
        rows = _rows(j * 64, 0, 64, 64)
        return (pltpu.make_async_copy(wqkv_hbm.at[rows, :], wqkv.at[rows, :], sems.at[j]),
                pltpu.make_async_copy(x_hbm.at[rows, :], xin.at[rows, :], sems.at[NH + j]))

    cp_o = pltpu.make_async_copy(wo_hbm, wo, sems.at[2 * NH])
    cp_g = pltpu.make_async_copy(wg_hbm, wgu.at[0], sems.at[2 * NH + 1])
    cp_u = pltpu.make_async_copy(wu_hbm, wgu.at[1], sems.at[2 * NH + 2])
    cp_d = pltpu.make_async_copy(wd_hbm, wd, sems.at[2 * NH + 3])
    cp_o.start()
    for j in range(NH):
        for cp in in_copies(j):
            cp.start()

    def x_col(c, parity):
        return (2 * parity + c // BC) * XB + c % BC * D

    cp_o.wait()
    for n in range(5):
        wn = min(128, D - 128 * n)
        blk = pltpu.bitcast(wo[:, 128 * n:128 * n + wn], u32)
        if wn < 128:
            blk = jnp.concatenate([blk, blk], axis=1)
        slab[n * D // 2:(n + 1) * D // 2, :] = blk
        rows = []
        for j in range(DH // 2):
            w2 = slab[pl.ds(n * D // 2 + j, H, stride=DH // 2), :]
            rows += [_unpack_lo(w2), _unpack_hi(w2)]
        rows = jnp.concatenate(rows, axis=0)
        for k, r0 in enumerate(KT):
            att[_rows(0, (15 + k) * D + 128 * n, wn), :] = rows[r0:r0 + 128].T[0:wn]

    @pl.loop(0, 5)
    def _(k):
        @pl.loop(2 * k, jnp.minimum(2 * k + 2, NH))
        def _(j):
            for cp in in_copies(j):
                cp.wait()

        r0 = jnp.minimum(k * 128, KT[-1])
        xslab[0:S // 2, :] = pltpu.bitcast(xin[_rows(r0, 0, 128, 64), :].T, u32)
        slab[0:3 * D // 2, :] = pltpu.bitcast(wqkv[_rows(r0, 0, 128, 64), :].T, u32)
        for c in range(NCOL):
            w2 = xslab[pl.ds(c, 128, stride=NCOL), :].T
            xs[_rows(r0, x_col(c, 0), 128), :] = _unpack_lo(w2)
            xs[_rows(r0, x_col(c, 1), 128), :] = _unpack_hi(w2)
        for s in range(3):
            for j in range(DH // 2):
                w2 = slab[pl.ds(s * (D // 2) + j, H, stride=DH // 2), :]
                att[_rows(k * D, 5 * s * D + 64 * j, 32), :] = _unpack_lo(w2)
                att[_rows(k * D, 5 * s * D + 64 * j + 32, 32), :] = _unpack_hi(w2)

    cp_g.start()
    cp_u.start()
    cp_d.start()

    @pl.loop(0, 4)
    def _(s):
        for r in range(0, NA, 16):
            _prep_weights(1, lambda i, k: att[_rows(s * 5 * D, k * D + NA * i + r, 16), :],
                          aa, aaz, _rows(s * NA, r, 16, 16))

    def piece_row(i):
        return (i % 2) * 64 + (i // 2) * 16

    def prep_ffn_weights():
        cp_g.wait()
        cp_u.wait()

        @pl.loop(0, F // 128 // PREP_UNROLL)
        def _(n):
            eye = lax.broadcasted_iota(jnp.int32, (128, 128), 0) == lax.broadcasted_iota(jnp.int32, (128, 128), 1)
            eye = eye.astype(f32).astype(bf16)
            for t in range(PREP_UNROLL):
                for which in range(2):
                    col = pl.ds(pl.multiple_of(n * PREP_UNROLL * 128, 128) + t * 128, 128)
                    head = lax.dot_general(eye, wgu[which, 0:512, col], (((1,), (1,)), ((), ())),
                                           preferred_element_type=f32)
                    src = [head[:, r0:r0 + 128] for r0 in KT[:4]] + [wgu[which, KT[4]:D, col].T.astype(f32)]
                    _prep_weights(2, lambda i, k: src[k][piece_row(i):piece_row(i) + 16],
                                  agu, aguz, _rows(n * PREP_UNROLL * 32, 32 * t + 16 * which, 16, 16))

        cp_d.wait()

        @pl.loop(0, ND // 16)
        def _(r):
            for u in range(F // 512):
                blocks = [[wd[_rows(16 * r, ND * x, 16, 16), pl.ds(512 * u + 128 * kb, 128)].astype(f32)
                           for kb in range(4)] for x in range(4)]
                for p, s in enumerate(_operands(A_TERMS, blocks)):
                    ad[p, u, _rows(16 * r, 0, 16, 16), :] = s.astype(bf16)

    def norm_stats(blk, paced):
        base = blk * XB

        def mean_of(tot):
            return jnp.broadcast_to(jnp.sum(tot, axis=0, keepdims=True) * (1.0 / D), (8, 128))

        for c in range(BC):
            tot = xs[_rows(base, c * D, 8), :]
            for r in range(8, D, 8):
                tot = tot + xs[_rows(base, c * D + r, 8), :]
            mean = mean_of(tot)
            xs[_rows(base, STAT0 + 16 * c, 8), :] = mean
            if paced:
                xs[XPAD:XPAD + 8, :] = mean
            tot = None
            for r in range(0, D, 8):
                xc = xs[_rows(base, c * D + r, 8), :] - mean
                tot = xc * xc if tot is None else tot + xc * xc
            rstd = lax.rsqrt(mean_of(tot) + 1e-5)
            xs[_rows(base, STAT0 + 16 * c + 8, 8), :] = rstd
            if paced:
                xs[XPAD:XPAD + 8, :] = rstd

    def normed(blk, scale):
        base = blk * XB
        cols = []
        for c in range(BC):
            x = xs[_rows(base, c * D, D), :].reshape(D // 8, 8, 128)
            mean, rstd = xs[_rows(base, STAT0 + 16 * c, 8), :], xs[_rows(base, STAT0 + 16 * c + 8, 8), :]
            cols.append(((x - mean) * (rstd * scale)).reshape(D, 128))
        return jnp.concatenate(cols, axis=1)

    def qkv_base(blk):
        return ((blk // 2) * (5 * NCOL) + (blk % 2) * BC) * D

    def qkv_proj(blk):
        base = qkv_base(blk)
        out = _matmul(aa, aaz, 0, 3 * NA, _prep_acts(1, normed(blk, 1.0)), ORDER_QKV)
        for i, o in enumerate(out):
            for c in range(BC):
                oc = o[:, 128 * c:128 * (c + 1)]
                row = c * D + NA * i
                att[_rows(base, row, NA), :] = oc[0:NA]
                for s in (1, 2):
                    val = oc[s * NA:(s + 1) * NA]
                    att[_rows(base, row + 2 * s * NCOL * D, NA), :] = val
                    att[_rows(base, row + (2 * s - 1) * NCOL * D, NA), :] = pltpu.roll(val, 1, 1)

    def window(j):
        return range(max(j, 0), min(j + W, BC))

    def attend_paced(blk):
        base = qkv_base(blk)
        steps = [0]

        def pace(val, every):
            steps[0] += 1
            if steps[0] % every == 0:
                att[_rows(blk % 2 * 8, PAD + 8 * (steps[0] % 16), 8), :] = val

        for h in range(0, H, 8):
            q = {}
            for j in range(1 - W, BC):
                acc = {}
                for d in range(DH):
                    k = att[_rows(base, (2 * NCOL + j) * D + H * d + h, 8), :]
                    for c in window(j):
                        if (c, d) not in q:
                            q[c, d] = att[_rows(base, c * D + H * d + h, 8), :]
                        acc[c] = q[c, d] * k if d == 0 else acc[c] + q[c, d] * k
                    pace(acc[c], 2)
                for c in window(j):
                    att[_rows(P0, 8 * (c * W + c - j), 8), :] = acc[c] * (DH ** -0.5)
            p = []
            for c in range(BC):
                p.append(_softmax([att[_rows(P0, 8 * (c * W + w), 8), :] for w in range(W)], (blk % 2) * BC, c))
                pace(p[c][-1], 1)
            for d in range(DH):
                acc = {}
                for j in range(1 - W, BC):
                    v = att[_rows(base, (4 * NCOL + j) * D + H * d + h, 8), :]
                    for c in window(j):
                        acc[c] = p[c][c - j] * v if c not in acc else acc[c] + p[c][c - j] * v
                    pace(acc[c], 1)
                for c in range(BC):
                    att[_rows(O0, c * D + H * d + h, 8), :] = acc[c]

    def attend_first():
        @pl.loop(0, H // 8)
        def _(n):
            logit = [[None] * W for _ in range(BC)]
            for d in range(DH):
                k = {j: att[_rows(n * 8, (2 * NCOL + j) * D + H * d, 8), :] for j in range(1 - W, BC)}
                for c in range(BC):
                    q = att[_rows(n * 8, c * D + H * d, 8), :]
                    for w in range(W):
                        logit[c][w] = q * k[c - w] if d == 0 else logit[c][w] + q * k[c - w]
            p = [_softmax([l * (DH ** -0.5) for l in logit[c]], 0, c) for c in range(BC)]
            for d in range(DH):
                v = {j: att[_rows(n * 8, (4 * NCOL + j) * D + H * d, 8), :] for j in range(1 - W, BC)}
                for c in range(BC):
                    acc = p[c][0] * v[c]
                    for w in range(1, W):
                        acc = acc + p[c][w] * v[c - w]
                    att[_rows(n * 8, O0 + c * D + H * d, 8), :] = acc

    def out_proj(blk):
        o = jnp.concatenate([att[_rows(O0, c * D, D), :] for c in range(BC)], axis=1)
        y = jnp.concatenate(_matmul(aa, aaz, 3 * NA, NA, _prep_acts(1, o), ORDER_OUT), axis=0)
        for c in range(BC):
            xs[_rows(blk * XB, c * D, D), :] += y[:, 128 * c:128 * (c + 1)]

    def ffn(i):
        blk = i % NBLK
        rhs = _prep_acts(2, normed(blk, 0.5))
        chunks, row = [], 0
        for n in GATE_UP_CHUNKS:
            gu = _matmul(agu, aguz, 32 * row, 32 * n, rhs, ORDER_GATE_UP)
            gu = [t.reshape(n, 2, 16, TB) for t in gu]
            chunks.append([(t[:, 1] + t[:, 1] * jnp.tanh(t[:, 0])).reshape(16 * n, TB) for t in gu])
            row += n
        xs[XPAD:XPAD + 8, :] = chunks[STATS_AFTER][1][0:8, 0:128]
        norm_stats((i + 3) % NBLK, True)
        att[PAD:PAD + 8, :] = chunks[ATTEND_AFTER][1][0:8, 0:128]
        attend_paced((i + 1) % NBLK)

        pieces = [jnp.concatenate([t[r] for t in chunks], axis=0) for r in sorted(range(8), key=piece_row)]
        h = [jnp.concatenate([t[16 * j:16 * (j + 1)] for j in range(kb, F // 128, 4) for t in pieces], axis=0)
             for kb in range(4)]
        quad = _quad([[t[:, 128 * c:128 * (c + 1)] for c in range(BC)] for t in h])
        outer = {}
        recent = [chunks[-1][5][0:8, 0:128]] * 3

        def down(p):
            if p // 7 not in outer:
                op, *which = B_TERMS[p // 7]
                m = op(*[quad[q] for q in which])
                outer[p // 7] = _quad([r[::-1] for r in m] if p // 7 + 1 in MIRRORED else m)
            op, first, *rest = B_TERMS[p % 7]
            zero = jnp.minimum(jnp.abs(recent[-3]), 0.0)
            first = (outer[p // 7][first][0][0].reshape(-1, 8, 128) + zero).reshape(F // 4, 128)
            b = op([[first]], *[outer[p // 7][q] for q in rest])[0][0]
            prod = _dot(_load_wide(ad, (p,), 0, ND), b.astype(bf16))
            recent.append(prod[0:8])
            return prod

        for x, ys in enumerate(_combine(down, 0, ORDER_DOWN, mirrored=MIRRORED)):
            for c, y in enumerate(ys):
                xs[_rows(blk * XB, c * D + ND * x, ND), :] += y

    @pl.loop(0, 2 * NBLK + 3)
    def _(n):
        @pl.when((n == 0) | (n > 2 * NBLK))
        def _():
            norm_stats(jnp.maximum(n - 3, 0) % NBLK, False)

        @pl.when(n == 2)
        def _():
            attend_first()

        @pl.when(n == 3)
        def _():
            prep_ffn_weights()

        @pl.when(n >= 3)
        def _():
            ffn(n - 3)

        @pl.when((n >= 2) & (n < 2 * NBLK + 2))
        def _():
            out_proj((n - 2) % NBLK)

        @pl.when(n < 2 * NBLK)
        def _():
            qkv_proj(n % NBLK)
            norm_stats(jnp.where(n < 2, n + 1, n - 2) % NBLK, True)

    def out_copy(k, half):
        rows = _rows(jnp.maximum(KT[-1] - k * 128, 0), 64 * half, 64, 64)
        return pltpu.make_async_copy(stage.at[k, 64 * half:64 * (half + 1), :], out_hbm.at[rows, :],
                                     sems.at[2 * k + half])

    @pl.loop(0, 5)
    def _(k):
        r0 = jnp.maximum(KT[-1] - k * 128, 0)
        for c in range(NCOL):
            even = _bf16_bits(xs[_rows(r0, x_col(c, 0), 128), :])
            odd = _bf16_bits(xs[_rows(r0, x_col(c, 1), 128), :])
            xslab[pl.ds(c, 128, stride=NCOL), :] = ((even >> 16) | odd).T
        stage[k] = pltpu.bitcast(xslab[0:S // 2, :], bf16).T
        out_copy(k, 0).start()

        @pl.when(k < 4)
        def _():
            out_copy(k, 1).start()

    for j in range(NH):
        out_copy(j // 2, j % 2).wait()


@jax.jit
def pallas_interleave_layers__sliding_local_dilated__glu_gated_glu__prompt_kernel(
    A_x: jax.Array,
    A_wqkv: jax.Array,
    A_wo: jax.Array,
    B_x: jax.Array,
    B_w_gate: jax.Array,
    B_w_up: jax.Array,
    B_w_down: jax.Array,
):
    del B_x
    any_spec = pl.BlockSpec(memory_space=pl.ANY)
    vmem = pltpu.VMEM
    out = pl.pallas_call(
        _kernel,
        out_shape=jax.ShapeDtypeStruct((D, S), bf16),
        in_specs=[any_spec] * 6,
        out_specs=any_spec,
        scratch_shapes=[
            vmem((D, S), bf16), vmem((D, 3 * D), bf16), vmem((D, D), bf16),
            vmem((2, D, F), bf16), vmem((D, F), bf16),
            pltpu.SemaphoreType.DMA((2 * NH + 4,)),
            vmem((5 * D // 2 + 8, 128), u32), vmem((S // 2 + 8, 128), u32), vmem((5, 128, S), bf16),
            vmem((2, 7, 2, D, 128), bf16), vmem((2, D, 128), bf16),
            vmem((2, 49, 1, F // 4, 128), bf16), vmem((4, F // 4, 128), bf16),
            vmem((49, F // 512, ND, 128), bf16),
            vmem((XPAD + 8, 128), f32), vmem((PAD + 8 * 17, 128), f32),
        ],
        compiler_params=pltpu.CompilerParams(vmem_limit_bytes=127 * 2**20),
    )(A_x[0].T, A_wqkv, A_wo, B_w_gate, B_w_up, B_w_down.T)
    return out.T[None]
```

```python
import jax
import jax.numpy as jnp
import numpy as np
from jax import lax
import jax.experimental.pallas as pl
import jax.experimental.pallas.tpu as pltpu

S, D, F = 2048, 576, 4608
H, DH, W = 32, 18, 8
NCOL = 8
BC = 4
TB = 128 * BC
NBLK = S // TB
KT = (0, 128, 256, 384, 448)
NA = ND = D // 4
NH = D // 64

ORDER_QKV = ("2435167r",)
ORDER_OUT = ("2435167",)
ORDER_GATE_UP = ("2435167r", "2435167")
ORDER_DOWN = ("2435167", "2514376")
GATE_UP_CHUNKS = (12, 4, 4, 4, 4, 4, 4)
ATTEND_AFTER, STATS_AFTER = 0, 5
NP = 6
PREP_AFTER = ((200,), (), (), (120,), (), (80, 360), (), (200,), (), (40, 280), (), (80, 320), (), (120,), (), ())

STAT0 = BC * D
XB = STAT0 + BC * 16
XPAD = NBLK * XB
O0 = 2 * 5 * NCOL * D
P0 = O0 + BC * D
PAD = P0 + BC * W * 8

f32 = jnp.float32
bf16 = jnp.bfloat16
u32 = jnp.uint32


def _dot(a, b):
    return jnp.dot(a, b, preferred_element_type=f32)


def _unpack_lo(w):
    return pltpu.bitcast(w << 16, f32)


def _unpack_hi(w):
    return pltpu.bitcast(w & np.uint32(0xFFFF0000), f32)


def _bf16_bits(x):
    return pltpu.bitcast(x.astype(bf16).astype(f32), u32)


def _rows(base, row, n, align=8):
    if isinstance(base, int):
        return pl.ds(base + row, n)
    return pl.ds(pl.multiple_of(base, align) + row, n)


def _load(ref, idx, row, n):
    return ref[(*idx, slice(row, row + n))]


def _load_wide(ref, idx, row, n):
    return jnp.concatenate([_load(ref, (*idx, k), row, n) for k in range(ref.shape[len(idx)])], axis=1)


def _madd(a, b):
    return [[x + y for x, y in zip(r, s)] for r, s in zip(a, b)]


def _msub(a, b):
    return [[x - y for x, y in zip(r, s)] for r, s in zip(a, b)]


def _first(a):
    return a


def _quad(m):
    n = len(m) // 2
    return ([r[:n] for r in m[:n]], [r[n:] for r in m[:n]], [r[:n] for r in m[n:]], [r[n:] for r in m[n:]])


A_TERMS = ((_madd, 0, 3), (_madd, 2, 3), (_first, 0), (_first, 3), (_madd, 0, 1), (_msub, 2, 0), (_msub, 1, 3))
B_TERMS = ((_madd, 0, 3), (_first, 0), (_msub, 1, 3), (_msub, 2, 0), (_first, 3), (_madd, 0, 1), (_madd, 2, 3))
C_TERMS = ({1: 1, 4: 1, 5: -1, 7: 1}, {3: 1, 5: 1}, {2: 1, 4: 1}, {1: 1, 2: -1, 3: 1, 6: 1})
MIRRORED = (2, 5, 6, 7)


def _operands(terms, m):
    if len(m) == 1:
        yield m[0][0]
        return
    quad = _quad(m)
    for op, *which in terms:
        yield from _operands(terms, op(*[quad[i] for i in which]))


def _combine(product, first, orders, addend=None, mirrored=()):
    if not orders:
        return [[product(first)]]
    order = [int(i) for i in orders[0][:7]]
    m = {i: _combine(product, first + (i - 1) * 7 ** (len(orders) - 1), orders[1:]) for i in order}
    for i in mirrored:
        m[i] = [row[::-1] for row in m[i]]
    out = []
    for q, terms in enumerate(C_TERMS):
        vals = [(terms[i], m[i]) for i in order if i in terms]
        if addend is not None:
            vals.insert(0, (1, _quad(addend)[q]))
        if orders[0].endswith("r"):
            vals.reverse()
        sign, acc = vals[0]
        for sg, v in vals[1:]:
            acc = _madd(acc, v) if sg == sign else _msub(acc, v) if sign == 1 else _msub(v, acc)
            sign = 1
        out.append(acc)
    return [r + s for r, s in zip(out[0], out[1])] + [r + s for r, s in zip(out[2], out[3])]


def _prep_weights(level, tile, a, az, rows):
    g = 2 ** level
    kt = 4 // g
    lo = lax.broadcasted_iota(jnp.int32, (16, 128), 1) < 64

    def own(x, ty, k):
        if k < 3:
            return tile(2 * x + ty, k)
        if ty == 0:
            return jnp.where(lo, tile(2 * x, 3), tile(2 * x, 3) - tile(2 * x + 1, 3))
        return jnp.where(lo, tile(2 * x + 1, 3), tile(2 * x + 1, 4) - tile(2 * x, 4))

    for x in range(g):
        az[x, rows, :] = jnp.where(lo, tile(2 * x + 1, 4), tile(2 * x, 4)).astype(bf16)
    for ty in range(2):
        for k in range(kt):
            blocks = [[own(x, ty, kb * kt + k) for kb in range(g)] for x in range(g)]
            for p, s in enumerate(_operands(A_TERMS, blocks)):
                a[ty, p, k, rows, :] = s.astype(bf16)


def _prep_acts(level, x):
    g = 2 ** level
    kg, tw = 512 // g, x.shape[1] // g

    def sums(starts, n):
        blocks = [[x[r:r + n, tw * t:tw * (t + 1)] for t in range(g)] for r in starts]
        return [s.astype(bf16) for s in _operands(B_TERMS, blocks)]

    head = sums([kg * kb for kb in range(g)], kg - 64)
    tails = [sums([kg * (kb + 1) - 64 for kb in range(g - 1)] + [last], 64) for last in (448, 512)]
    return [[jnp.concatenate([a, b], axis=0) for a, b in zip(head, tail)] for tail in tails], x[448:576].astype(bf16)


def _matmul(a, az, row, n, rhs, orders, hook=_first):
    g = 2 ** len(orders)
    b, bz = rhs
    tw = bz.shape[1] // g
    shared = [hook(_dot(_load(az, (x,), row, n), bz)) for x in range(g)]
    shared = [[z[:, tw * t:tw * (t + 1)] for t in range(g)] for z in shared]
    out = [_combine(lambda p: hook(_dot(_load_wide(a, (ty, p), row, n), b[ty][p])), 0, orders, shared)
           for ty in range(2)]
    return [jnp.concatenate(out[ty][x], axis=1) for x in range(g) for ty in range(2)]


def _fold(x):
    return jnp.sum(x.reshape(-1, 8, 128), axis=0)


def _mean(tot):
    return jnp.broadcast_to(jnp.sum(tot, axis=0, keepdims=True) * (1.0 / D), (8, 128))


def _softmax(logit, first_col, c):
    pos = lax.broadcasted_iota(jnp.int32, (8, 128), 1) * NCOL + first_col
    logit = [l if w <= c else jnp.where(pos >= w - c, l, -1e9) for w, l in enumerate(logit)]
    top = logit[0]
    for l in logit[1:]:
        top = jnp.maximum(top, l)
    e = [jnp.exp(l - top) for l in logit]
    den = e[0]
    for x in e[1:]:
        den = den + x
    inv = 1.0 / den
    return [x * inv for x in e]


def _kernel(x_hbm, wqkv_hbm, wo_hbm, wg_hbm, wu_hbm, wd_hbm, out_hbm,
            xin, wqkv, wo, wgu, wd, sems, slab, xslab, stage,
            aa, aaz, agu, aguz, ad, xs, att):

    def in_copies(j):
        rows = _rows(j * 64, 0, 64, 64)
        return (pltpu.make_async_copy(wqkv_hbm.at[rows, :], wqkv.at[rows, :], sems.at[j]),
                pltpu.make_async_copy(x_hbm.at[rows, :], xin.at[rows, :], sems.at[NH + j]))

    cp_o = pltpu.make_async_copy(wo_hbm, wo, sems.at[2 * NH])
    cp_d = pltpu.make_async_copy(wd_hbm, wd, sems.at[2 * NH + 1])

    def gate_up_copies(n):
        cols = _rows(n * (F // NP), 0, F // NP, 128)
        return [pltpu.make_async_copy(src.at[:, cols], wgu.at[which, :, cols], sems.at[2 * NH + 2 + n])
                for which, src in enumerate((wg_hbm, wu_hbm))]

    cp_o.start()
    for j in range(NH):
        for cp in in_copies(j):
            cp.start()

    def x_col(c, parity):
        return (2 * parity + c // BC) * XB + c % BC * D

    sum_rows = {(c, t): (2 * t + c // BC) * XB + STAT0 + 16 * (c % BC) for c in range(NCOL) for t in range(2)}
    for row in sum_rows.values():
        xs[row:row + 8, :] = jnp.zeros((8, 128), f32)

    cp_o.wait()
    for n in range(5):
        wn = min(128, D - 128 * n)
        blk = pltpu.bitcast(wo[:, 128 * n:128 * n + wn], u32)
        if wn < 128:
            blk = jnp.concatenate([blk, blk], axis=1)
        slab[n * D // 2:(n + 1) * D // 2, :] = blk
        rows = []
        for j in range(DH // 2):
            w2 = slab[pl.ds(n * D // 2 + j, H, stride=DH // 2), :]
            rows += [_unpack_lo(w2), _unpack_hi(w2)]
        rows = jnp.concatenate(rows, axis=0)
        for k, r0 in enumerate(KT):
            att[_rows(0, (15 + k) * D + 128 * n, wn), :] = rows[r0:r0 + 128].T[0:wn]

    def prep_attn_weights(s):
        for r in range(0, NA, 16):
            _prep_weights(1, lambda i, k: att[_rows(s * 5 * D, k * D + NA * i + r, 16), :],
                          aa, aaz, _rows(s * NA, r, 16, 16))

    prep_attn_weights(3)

    @pl.loop(0, 5)
    def _(k):
        @pl.loop(2 * k, jnp.minimum(2 * k + 2, NH))
        def _(j):
            for cp in in_copies(j):
                cp.wait()

        @pl.when(k == 3)
        def _():
            for cp in gate_up_copies(0):
                cp.start()

        r0 = jnp.minimum(k * 128, KT[-1])
        tot = {key: xs[row:row + 8, :] for key, row in sum_rows.items()}
        xslab[0:S // 2, :] = pltpu.bitcast(xin[_rows(r0, 0, 128, 64), :].T, u32)
        slab[0:3 * D // 2, :] = pltpu.bitcast(wqkv[_rows(r0, 0, 128, 64), :].T, u32)
        for c in range(NCOL):
            w2 = xslab[pl.ds(c, 128, stride=NCOL), :].T
            for t, val in enumerate((_unpack_lo(w2), _unpack_hi(w2))):
                xs[_rows(r0, x_col(c, t), 128), :] = val
                tot[c, t] = tot[c, t] + _fold(val[64:]) + jnp.where(k < 4, _fold(val[:64]), 0.0)
        for key, row in sum_rows.items():
            xs[row:row + 8, :] = tot[key]
        for s in range(3):
            for j in range(DH // 2):
                w2 = slab[pl.ds(s * (D // 2) + j, H, stride=DH // 2), :]
                att[_rows(k * D, 5 * s * D + 64 * j, 32), :] = _unpack_lo(w2)
                att[_rows(k * D, 5 * s * D + 64 * j + 32, 32), :] = _unpack_hi(w2)

    pl.loop(0, 3)(prep_attn_weights)

    def piece_row(i):
        return (i % 2) * 64 + (i // 2) * 16

    def prep_down_weights():
        cp_d.wait()

        @pl.loop(0, ND // 16)
        def _(r):
            for u in range(F // 512):
                blocks = [[wd[_rows(16 * r, ND * x, 16, 16), pl.ds(512 * u + 128 * kb, 128)].astype(f32)
                           for kb in range(4)] for x in range(4)]
                for p, s in enumerate(_operands(A_TERMS, blocks)):
                    ad[p, u, _rows(16 * r, 0, 16, 16), :] = s.astype(bf16)

    def norm_stats(blk, paced, first=0, count=BC):
        base, stat = blk * XB + first * D, blk * XB + first * 16

        for c in range(count):
            mean = _mean(xs[_rows(stat, STAT0 + 16 * c, 8), :])
            tot = None
            for r in range(0, D, 8):
                xc = xs[_rows(base, c * D + r, 8), :] - mean
                tot = xc * xc if tot is None else tot + xc * xc
            rstd = lax.rsqrt(_mean(tot) + 1e-5)
            xs[_rows(stat, STAT0 + 16 * c + 8, 8), :] = rstd
            if paced:
                xs[XPAD:XPAD + 8, :] = rstd

    def normed(blk, scale, first=0, count=BC):
        base, stat = blk * XB + first * D, blk * XB + first * 16
        cols = []
        for c in range(count):
            x = xs[_rows(base, c * D, D), :].reshape(D // 8, 8, 128)
            tot, rstd = xs[_rows(stat, STAT0 + 16 * c, 8), :], xs[_rows(stat, STAT0 + 16 * c + 8, 8), :]
            cols.append(((x - _mean(tot)) * (rstd * scale)).reshape(D, 128))
        return jnp.concatenate(cols, axis=1)

    def qkv_base(blk):
        return ((blk // 2) * (5 * NCOL) + (blk % 2) * BC) * D

    def qkv_proj(blk, first, count, hook=_first):
        base = qkv_base(blk) + first * D
        out = _matmul(aa, aaz, 0, 3 * NA, _prep_acts(1, normed(blk, 1.0, first, count)), ORDER_QKV, hook)
        for i, o in enumerate(out):
            for c in range(count):
                oc = o[:, 128 * c:128 * (c + 1)]
                row = c * D + NA * i
                att[_rows(base, row, NA), :] = oc[0:NA]
                for s in (1, 2):
                    val = oc[s * NA:(s + 1) * NA]
                    att[_rows(base, row + 2 * s * NCOL * D, NA), :] = val
                    att[_rows(base, row + (2 * s - 1) * NCOL * D, NA), :] = pltpu.roll(val, 1, 1)

    def window(j):
        return range(max(j, 0), min(j + W, BC))

    def attend_paced(blk):
        base = qkv_base(blk)
        steps = [0]

        def pace(val, every):
            steps[0] += 1
            if steps[0] % every == 0:
                att[_rows(blk % 2 * 8, PAD + 8 * (steps[0] % 16), 8), :] = val

        for h in range(0, H, 8):
            q = {}
            for j in range(1 - W, BC):
                acc = {}
                for d in range(DH):
                    k = att[_rows(base, (2 * NCOL + j) * D + H * d + h, 8), :]
                    for c in window(j):
                        if (c, d) not in q:
                            q[c, d] = att[_rows(base, c * D + H * d + h, 8), :]
                        acc[c] = q[c, d] * k if d == 0 else acc[c] + q[c, d] * k
                    pace(acc[c], 2)
                for c in window(j):
                    att[_rows(P0, 8 * (c * W + c - j), 8), :] = acc[c] * (DH ** -0.5)
            p = []
            for c in range(BC):
                p.append(_softmax([att[_rows(P0, 8 * (c * W + w), 8), :] for w in range(W)], (blk % 2) * BC, c))
                pace(p[c][-1], 1)
            for d in range(DH):
                acc = {}
                for j in range(1 - W, BC):
                    v = att[_rows(base, (4 * NCOL + j) * D + H * d + h, 8), :]
                    for c in window(j):
                        acc[c] = p[c][c - j] * v if c not in acc else acc[c] + p[c][c - j] * v
                    pace(acc[c], 1)
                for c in range(BC):
                    att[_rows(O0, c * D + H * d + h, 8), :] = acc[c]

    def attend_first():
        @pl.loop(0, H // 8)
        def _(n):
            logit = [[None] * W for _ in range(BC)]
            for d in range(DH):
                k = {j: att[_rows(n * 8, (2 * NCOL + j) * D + H * d, 8), :] for j in range(1 - W, BC)}
                for c in range(BC):
                    q = att[_rows(n * 8, c * D + H * d, 8), :]
                    for w in range(W):
                        logit[c][w] = q * k[c - w] if d == 0 else logit[c][w] + q * k[c - w]
            p = [_softmax([l * (DH ** -0.5) for l in logit[c]], 0, c) for c in range(BC)]
            for d in range(DH):
                v = {j: att[_rows(n * 8, (4 * NCOL + j) * D + H * d, 8), :] for j in range(1 - W, BC)}
                for c in range(BC):
                    acc = p[c][0] * v[c]
                    for w in range(1, W):
                        acc = acc + p[c][w] * v[c - w]
                    att[_rows(n * 8, O0 + c * D + H * d, 8), :] = acc

    def add_to_residual(blk, y):
        for c in range(BC):
            sums = []
            for i in range(4):
                rows = _rows(blk * XB, c * D + D // 4 * i, D // 4)
                new = xs[rows, :] + y[i][c]
                xs[rows, :] = new
                sums.append(_fold(new))
            xs[_rows(blk * XB, STAT0 + 16 * c, 8), :] = (sums[0] + sums[1]) + (sums[2] + sums[3])

    def out_proj(blk):
        o = jnp.concatenate([att[_rows(O0, c * D, D), :] for c in range(BC)], axis=1)
        y = _matmul(aa, aaz, 3 * NA, NA, _prep_acts(1, o), ORDER_OUT)
        add_to_residual(blk, [[t[:, 128 * c:128 * (c + 1)] for c in range(BC)] for t in y])

    def ffn(i):
        blk = i % NBLK
        rhs = _prep_acts(2, normed(blk, 0.5))
        chunks, row = [], 0
        for n in GATE_UP_CHUNKS:
            gu = _matmul(agu, aguz, 32 * row, 32 * n, rhs, ORDER_GATE_UP)
            gu = [t.reshape(n, 2, 16, TB) for t in gu]
            chunks.append([(t[:, 1] + t[:, 1] * jnp.tanh(t[:, 0])).reshape(16 * n, TB) for t in gu])
            row += n
        xs[XPAD:XPAD + 8, :] = chunks[STATS_AFTER][1][0:8, 0:128]
        norm_stats((i + 3) % NBLK, True)
        att[PAD:PAD + 8, :] = chunks[ATTEND_AFTER][1][0:8, 0:128]
        attend_paced((i + 1) % NBLK)

        pieces = [jnp.concatenate([t[r] for t in chunks], axis=0) for r in sorted(range(8), key=piece_row)]
        h = [jnp.concatenate([t[16 * j:16 * (j + 1)] for j in range(kb, F // 128, 4) for t in pieces], axis=0)
             for kb in range(4)]
        quad = _quad([[t[:, 128 * c:128 * (c + 1)] for c in range(BC)] for t in h])
        outer = {}
        recent = [chunks[-1][5][0:8, 0:128]] * 3

        def down(p):
            if p // 7 not in outer:
                op, *which = B_TERMS[p // 7]
                m = op(*[quad[q] for q in which])
                outer[p // 7] = _quad([r[::-1] for r in m] if p // 7 + 1 in MIRRORED else m)
            op, first, *rest = B_TERMS[p % 7]
            zero = jnp.minimum(jnp.abs(recent[-3]), 0.0)
            first = (outer[p // 7][first][0][0].reshape(-1, 8, 128) + zero).reshape(F // 4, 128)
            b = op([[first]], *[outer[p // 7][q] for q in rest])[0][0]
            prod = _dot(_load_wide(ad, (p,), 0, ND), b.astype(bf16))
            recent.append(prod[0:8])
            return prod

        add_to_residual(blk, _combine(down, 0, ORDER_DOWN, mirrored=MIRRORED))

    def first_qkv(n):
        @pl.when(n + 1 < NP)
        def _():
            for cp in gate_up_copies(n + 1):
                cp.start()

        @pl.when(n + 1 == NP)
        def _():
            cp_d.start()

        for cp in gate_up_copies(n):
            cp.wait()
        tiles = F // 128 // NP
        todo = [(t, which) for t in range(tiles) for which in range(2)]

        def prep(after=None):
            t, which = todo.pop(0)
            src = [wgu[which, r0:r0 + 128, _rows(n * tiles * 128, t * 128, 128, 128)] for r0 in KT]
            if after is not None:
                zero = pltpu.bitcast(jnp.minimum(jnp.abs(after), 0.0), u32)
                src = [jnp.concatenate([pltpu.bitcast(pltpu.bitcast(b[0:16], u32) | zero, bf16), b[16:]], axis=0)
                       for b in src]
            src = [b.T.astype(f32) for b in src]
            _prep_weights(2, lambda i, k: src[k][piece_row(i):piece_row(i) + 16],
                          agu, aguz, _rows(n * tiles * 32, 32 * t + 16 * which, 16, 16))

        plan = list(PREP_AFTER)
        prep()
        prep()

        def hook(m):
            for row in plan.pop(0):
                prep(m[row:row + 8, 0:128])
            return m

        qkv_proj(n // 2, (n % 2) * 2, 2, hook)
        assert not todo

    @pl.loop(0, 2 * NBLK + 3)
    def _(n):
        @pl.when((n <= 3) | (n > 2 * NBLK))
        def _():
            norm_stats(jnp.where(n < 3, n, n - 3) % NBLK, False)

        @pl.when(n < 3)
        def _():
            pl.loop(2 * n, 2 * n + 2)(first_qkv)

        @pl.when(n == 2)
        def _():
            attend_first()

        @pl.when(n == 3)
        def _():
            prep_down_weights()

        @pl.when(n >= 3)
        def _():
            ffn(n - 3)

        @pl.when((n >= 2) & (n < 2 * NBLK + 2))
        def _():
            out_proj((n - 2) % NBLK)

        @pl.when((n >= 3) & (n < 2 * NBLK))
        def _():
            @pl.loop(0, 2)
            def _(half):
                qkv_proj(n % NBLK, 2 * half, 2)
                norm_stats((n - 2) % NBLK, True, 2 * half, 2)

    def out_copy(k, half):
        rows = _rows((max if isinstance(k, int) else jnp.maximum)(KT[-1] - k * 128, 0), 64 * half, 64, 64)
        return pltpu.make_async_copy(stage.at[k, 64 * half:64 * (half + 1), :], out_hbm.at[rows, :],
                                     sems.at[2 * k + half])

    @pl.loop(0, 5)
    def _(k):
        r0 = jnp.maximum(KT[-1] - k * 128, 0)
        for c in range(NCOL):
            even = _bf16_bits(xs[_rows(r0, x_col(c, 0), 128), :])
            odd = _bf16_bits(xs[_rows(r0, x_col(c, 1), 128), :])
            xslab[pl.ds(c, 128, stride=NCOL), :] = ((even >> 16) | odd).T
        stage[k] = pltpu.bitcast(xslab[0:S // 2, :], bf16).T
        out_copy(k, 0).start()

        @pl.when(k < 4)
        def _():
            out_copy(k, 1).start()

    for j in range(NH):
        out_copy(j // 2, j % 2).wait()


@jax.jit
def pallas_interleave_layers__sliding_local_dilated__glu_gated_glu__prompt_kernel(
    A_x: jax.Array,
    A_wqkv: jax.Array,
    A_wo: jax.Array,
    B_x: jax.Array,
    B_w_gate: jax.Array,
    B_w_up: jax.Array,
    B_w_down: jax.Array,
):
    del B_x
    any_spec = pl.BlockSpec(memory_space=pl.ANY)
    vmem = pltpu.VMEM
    out = pl.pallas_call(
        _kernel,
        out_shape=jax.ShapeDtypeStruct((D, S), bf16),
        in_specs=[any_spec] * 6,
        out_specs=any_spec,
        scratch_shapes=[
            vmem((D, S), bf16), vmem((D, 3 * D), bf16), vmem((D, D), bf16),
            vmem((2, D, F), bf16), vmem((D, F), bf16),
            pltpu.SemaphoreType.DMA((2 * NH + 2 + NP,)),
            vmem((5 * D // 2 + 8, 128), u32), vmem((S // 2 + 8, 128), u32), vmem((5, 128, S), bf16),
            vmem((2, 7, 2, D, 128), bf16), vmem((2, D, 128), bf16),
            vmem((2, 49, 1, F // 4, 128), bf16), vmem((4, F // 4, 128), bf16),
            vmem((49, F // 512, ND, 128), bf16),
            vmem((XPAD + 8, 128), f32), vmem((PAD + 8 * 17, 128), f32),
        ],
        compiler_params=pltpu.CompilerParams(vmem_limit_bytes=127 * 2**20),
    )(A_x[0].T, A_wqkv, A_wo, B_w_gate, B_w_up, B_w_down.T)
    return out.T[None]
```
